```python
import jax
import jax.numpy as jnp

def _softmax(x, axis=-1):
    return jax.nn.softmax(x, axis=axis)

def _gelu(x):
    return jax.nn.gelu(x, approximate=True)

def _silu(x):
    return jax.nn.silu(x)

def _sigmoid(x):
    return jax.nn.sigmoid(x)

def _layernorm(x, axis=-1, eps=1e-05):
    m = jnp.mean(x, axis=axis, keepdims=True)
    v = jnp.var(x, axis=axis, keepdims=True)
    return (x - m) / jnp.sqrt(v + eps)

def _scatter_add(tgt, idx, src, axis=0):
    return tgt.at[idx].add(src)

def _segment_sum(src, seg, n):
    return jax.ops.segment_sum(src, seg, n)

class _Rng:

    def __init__(self, key):
        self._k = key

    def _next(self):
        self._k, sub = jax.random.split(self._k)
        return sub

    def normal(self, shape):
        return jax.random.normal(self._next(), shape, dtype=jnp.bfloat16)

    def randint(self, lo, hi, shape):
        return jax.random.randint(self._next(), shape, lo, hi, dtype=jnp.int32)

    def uniform(self, shape, lo=0.0, hi=1.0):
        return jax.random.uniform(self._next(), shape, jnp.bfloat16, lo, hi)

    def permutation(self, n):
        return jax.random.permutation(self._next(), n)
kernel_name = 'adaLN_cond__sliding_local_dilated__glu_gated_swiglu__prompt'

def setup_inputs():
    _rng = _Rng(jax.random.key(int.from_bytes(__import__("os").urandom(4), "little")))
    _w = lambda a: (lambda t: t.astype(jnp.bfloat16) if jnp.issubdtype(t.dtype, jnp.floating) else t)(jnp.asarray(a))

    def _A_setup():
        B, S, D = (1, 2048, 1024)
        return {'x': _w((lambda *s: _rng.normal(s) * 0.05)(B, S, D)), 'wqkv': _w((lambda *s: _rng.normal(s) * 0.05)(D, 3 * D)), 'wo': _w((lambda *s: _rng.normal(s) * 0.05)(D, D))}
    _A_in = _A_setup()

    def _B_setup():
        B, S, D, F = (1, 2048, 1024, 3584)
        return {'x': _w((lambda *s: _rng.normal(s) * 0.05)(B, S, D)), 'w1': _w((lambda *s: _rng.normal(s) * 0.05)(D, F) * (2.0 / D) ** 0.5), 'w3': _w((lambda *s: _rng.normal(s) * 0.05)(D, F) * (2.0 / D) ** 0.5), 'w2': _w((lambda *s: _rng.normal(s) * 0.05)(F, D) * (2.0 / F) ** 0.5)}
    _B_in = _B_setup()
    return {'A_x': _A_in['x'], 'A_wqkv': _A_in['wqkv'], 'A_wo': _A_in['wo'], 'B_x': _B_in['x'], 'B_w1': _B_in['w1'], 'B_w3': _B_in['w3'], 'B_w2': _B_in['w2'], 'c': _w((lambda *s: _rng.normal(s) * 0.05)(1, 1024)), 'w_mod': _w((lambda *s: _rng.normal(s) * 0.05)(1024, 6 * 1024) * 1024 ** (-0.5))}

def reference(A_x, A_wqkv, A_wo, B_x, B_w1, B_w3, B_w2, c, w_mod):

    def _A_ref(x, wqkv, wo):
        B, S, D = x.shape
        H = 32
        Dh = D // H
        W, dil = (8, 2)
        qkv = (lambda x, *d: x.transpose(*d))((x @ wqkv).reshape(B, S, 3, H, Dh), 2, 0, 3, 1, 4)
        q, k, v = (qkv[0], qkv[1], qkv[2])
        scale = Dh ** (-0.5)
        pos = jnp.arange(S)
        off = jnp.arange(W) * dil
        idx = pos[:, None] - off[None, :]
        mask = idx >= 0
        idx_c = jnp.where(mask, idx, 0).reshape(-1)
        kg = k[:, :, idx_c, :].reshape(B, H, S, W, Dh)
        vg = v[:, :, idx_c, :].reshape(B, H, S, W, Dh)
        logits = jnp.einsum('bhsd,bhswd->bhsw', q, kg) * scale
        logits = jnp.where(mask[None, None, :, :], logits, -1000000000.0)
        attn = _softmax(logits, axis=-1)
        o = jnp.einsum('bhsw,bhswd->bhsd', attn, vg)
        return (lambda x, *d: x.transpose(*d))(o, 0, 2, 1, 3).reshape(B, S, D) @ wo

    def _B_ref(x, w1, w3, w2):
        gate = jnp.einsum('bsd,df->bsf', x, w1)
        up = jnp.einsum('bsd,df->bsf', x, w3)
        h = _silu(gate) * up
        out = jnp.einsum('bsf,fd->bsd', h, w2)
        return out
    x = A_x
    mod = (_silu(c) @ w_mod).reshape(c.shape[0], 6, 1, -1)
    sa, ca, ga, sb, cb, gb = (mod[:, 0].copy(), mod[:, 1].copy(), mod[:, 2].copy(), mod[:, 3].copy(), mod[:, 4].copy(), mod[:, 5].copy())
    h = _layernorm(x, axis=-1) * (1 + ca) + sa
    x = x + ga * _A_ref(h, A_wqkv, A_wo)
    h = _layernorm(x, axis=-1) * (1 + cb) + sb
    x = x + gb * _B_ref(h, B_w1, B_w3, B_w2)
    return x
```

```python
import functools
import numpy as np
import jax
import jax.numpy as jnp
from jax import lax
from jax.experimental import pallas as pl
from jax.experimental.pallas import tpu as pltpu

S, D, H, DH, F = 2048, 1024, 32, 32, 3584
W, DIL = 8, 2
HALO = 16
f32, bf16, i32 = jnp.float32, jnp.bfloat16, jnp.int32


def _ln_mod(xf, a, b):
    mean = jnp.sum(xf, axis=-1, keepdims=True) * (1.0 / D)
    xc = xf - mean
    var = jnp.sum(xc * xc, axis=-1, keepdims=True) * (1.0 / D)
    inv = lax.rsqrt(var + 1e-5)
    return (xc * inv) * a + b


def _xor_net(vs, masks):
    vs = list(vs)
    for b in range(3):
        nv = list(vs)
        for u in range(8):
            if not (u >> b) & 1:
                p = u | (1 << b)
                nv[u] = jnp.where(masks[b], vs[p], vs[u])
                nv[p] = jnp.where(masks[b], vs[u], vs[p])
        vs = nv
    return vs


def _perm_consts():
    lane = lax.broadcasted_iota(i32, (8, 128), 1)
    m_in = [((lane >> (2 + b)) & 1) == 1 for b in range(3)]
    r, j, a = lane >> 5, (lane >> 2) & 7, lane & 3
    idx = [a * 32 + (j ^ u) * 4 + r for u in range(8)]
    return m_in, idx


def _permute_cols(w_ref, col0):
    masks, idx = _perm_consts()
    for g in range(D // 16):
        rows = pl.ds(g * 16, 16)
        src = [pltpu.bitcast(w_ref[rows, col0 + j * 128:col0 + (j + 1) * 128], i32) for j in range(8)]
        mer = _xor_net(src, masks)
        per = [jnp.take_along_axis(mer[u], idx[u], axis=1) for u in range(8)]
        dst = _xor_net(per, masks)
        for t in range(8):
            w_ref[rows, col0 + t * 128:col0 + (t + 1) * 128] = pltpu.bitcast(dst[t], bf16)


def _permute_rows(src_ref, dst_ref):
    for j in range(8):
        for dp in range(16):
            A = src_ref[j, pl.ds(dp, 16, stride=32), :]
            B = src_ref[j, pl.ds(16 + dp, 16, stride=32), :]
            lo = (A & 0xFFFF) | (B << 16)
            hi = lax.shift_right_logical(A, 16) | (B & jnp.int32(-65536))
            for e, val in enumerate((lo, hi)):
                d = 2 * dp + e
                dst_ref[pl.ds(d * 32, 32), j * 128:(j + 1) * 128] = pltpu.bitcast(val, bf16)


def _attn(q, kv_ref, M, pos0):
    scale = DH ** -0.5
    pos = pos0 + lax.broadcasted_iota(i32, (M, 128), 0)
    logits = []
    for w in range(W):
        acc = None
        for j in range(8):
            kk = kv_ref[j, pl.ds(HALO - DIL * w, M), :]
            p = q[:, j * 128:(j + 1) * 128] * kk
            acc = p if acc is None else acc + p
        acc = acc + pltpu.roll(acc, 64, 1)
        acc = acc + pltpu.roll(acc, 32, 1)
        acc = acc * scale
        if w > 0:
            acc = jnp.where(pos >= DIL * w, acc, -1e9)
        logits.append(acc)
    m = logits[0]
    for w in range(1, W):
        m = jnp.maximum(m, logits[w])
    es = [jnp.exp(l - m) for l in logits]
    den = es[0]
    for w in range(1, W):
        den = den + es[w]
    inv = 1.0 / den
    outs = []
    for j in range(8):
        acc = None
        for w in range(W):
            vv = kv_ref[8 + j, pl.ds(HALO - DIL * w, M), :]
            p = es[w] * vv
            acc = p if acc is None else acc + p
        outs.append((acc * inv).astype(bf16))
    return jnp.concatenate(outs, axis=1)


def make_kernel(TM, FC, debug):
    NT = S // TM

    def kernel(x_hbm, wqkv_hbm, wo_hbm, w1_hbm, w3_hbm, w2_hbm, c_hbm, wmod_hbm, out_hbm,
               x_v, wqkv_v, wo_raw, wo_v, w1_v, w3_v, w2_v, c_v, wma_v, wmb_v, wmc_v,
               mod_v, h_v, kv_v, x1_v, out_v, sems, osem):
        def cp(src, dst, k):
            return pltpu.make_async_copy(src, dst, sems.at[k])

        cps = {
            'c': cp(c_hbm, c_v, 0),
            'wma': cp(wmod_hbm.at[:, 0:2 * D], wma_v, 1),
            'x0': cp(x_hbm.at[0:TM], x_v.at[0:TM], 2),
            'wq': cp(wqkv_hbm.at[:, 0:D], wqkv_v.at[:, 0:D], 3),
            'wk': cp(wqkv_hbm.at[:, D:2 * D], wqkv_v.at[:, D:2 * D], 4),
            'wv': cp(wqkv_hbm.at[:, 2 * D:3 * D], wqkv_v.at[:, 2 * D:3 * D], 5),
            'wmb': cp(wmod_hbm.at[:, 2 * D:3 * D], wmb_v, 6),
            'xr': cp(x_hbm.at[TM:S], x_v.at[TM:S], 7),
            'wmc': cp(wmod_hbm.at[:, 3 * D:6 * D], wmc_v, 8),
            'w1': cp(w1_hbm, w1_v, 9),
            'w3': cp(w3_hbm, w3_v, 10),
            'w2': cp(w2_hbm, w2_v, 11),
        }
        wo_cps = [cp(wo_hbm.at[:, j * 128:(j + 1) * 128], wo_raw.at[j], 12 + j) for j in range(8)]
        for k in ('c', 'wma', 'x0', 'wq', 'wk', 'wv'):
            cps[k].start()
        for c_ in wo_cps:
            c_.start()
        for k in ('wmb', 'xr', 'wmc', 'w1', 'w3', 'w2'):
            cps[k].start()

        kv_v[:, 0:HALO, :] = jnp.zeros((16, HALO, 128), f32)

        cps['c'].wait()
        cf = c_v[...].astype(f32)
        sc = (cf * jax.nn.sigmoid(cf)).astype(bf16)
        sc = jnp.broadcast_to(sc, (16, D))

        def mod_part(w_ref, col0, n, plus_one):
            for p in range(n):
                r = jnp.dot(sc, w_ref[:, p * D:(p + 1) * D], preferred_element_type=f32)[0:8]
                if plus_one[p]:
                    r = r + 1.0
                mod_v[:, col0 + p * D:col0 + (p + 1) * D] = r

        cps['wma'].wait()
        mod_part(wma_v, 0, 2, (False, True))

        def mod(k):
            return mod_v[0:1, k * D:(k + 1) * D]

        def ln1(t):
            r = pl.ds(pl.multiple_of(t * TM, TM), TM)
            h_v[...] = _ln_mod(x_v[r, :].astype(f32), mod(1), mod(0)).astype(bf16)

        cps['x0'].wait()
        ln1(0)

        def a_body(i, first):
            h = h_v[...]
            r = pl.ds(pl.multiple_of(i * TM, TM), TM)
            if first:
                cps['wq'].wait()
                _permute_cols(wqkv_v, 0)
                cps['wk'].wait()
                _permute_cols(wqkv_v, D)
            q = jnp.dot(h, wqkv_v[:, 0:D], preferred_element_type=f32)
            if first:
                cps['wv'].wait()
                _permute_cols(wqkv_v, 2 * D)
            k = jnp.dot(h, wqkv_v[:, D:2 * D], preferred_element_type=f32)
            for j in range(8):
                kv_v[j, HALO:HALO + TM, :] = k[:, j * 128:(j + 1) * 128]
            if first:
                for c_ in wo_cps:
                    c_.wait()
                _permute_rows(wo_raw.bitcast(i32), wo_v)
            v = jnp.dot(h, wqkv_v[:, 2 * D:3 * D], preferred_element_type=f32)
            for j in range(8):
                kv_v[8 + j, HALO:HALO + TM, :] = v[:, j * 128:(j + 1) * 128]
            o = _attn(q, kv_v, TM, i * TM)
            kv_v[:, 0:HALO, :] = kv_v[:, TM:TM + HALO, :]
            y = jnp.dot(o, wo_v[...], preferred_element_type=f32)
            if first:
                cps['wmb'].wait()
                mod_part(wmb_v, 2 * D, 1, (False,))
                cps['xr'].wait()
            x1_v[r, :] = x_v[r, :].astype(f32) + mod(2) * y
            ln1(jnp.minimum(i + 1, NT - 1))

        a_body(0, True)

        def a_loop(i, carry):
            a_body(i, False)
            return carry
        lax.fori_loop(1, NT, a_loop, 0)

        cps['wmc'].wait()
        mod_part(wmc_v, 3 * D, 3, (False, True, False))
        cps['w1'].wait()
        cps['w3'].wait()
        cps['w2'].wait()

        def ln2(t):
            r = pl.ds(pl.multiple_of(t * TM, TM), TM)
            h_v[...] = _ln_mod(x1_v[r, :], mod(4), mod(3)).astype(bf16)

        ln2(0)

        def f_loop(i, carry):
            r = pl.ds(pl.multiple_of(i * TM, TM), TM)
            h2 = h_v[...]
            acc = None
            for c in range(F // FC):
                g = jnp.dot(h2, w1_v[:, c * FC:(c + 1) * FC], preferred_element_type=f32)
                u = jnp.dot(h2, w3_v[:, c * FC:(c + 1) * FC], preferred_element_type=f32)
                a = (g * jax.nn.sigmoid(g) * u).astype(bf16)
                d = jnp.dot(a, w2_v[c * FC:(c + 1) * FC, :], preferred_element_type=f32)
                acc = d if acc is None else acc + d
            out_v[r, :] = (x1_v[r, :] + mod(5) * acc).astype(out_v.dtype)
            ln2(jnp.minimum(i + 1, NT - 1))
            pltpu.make_async_copy(out_v.at[r], out_hbm.at[r], osem.at[i]).start()
            return carry
        lax.fori_loop(0, NT, f_loop, 0)
        for i in range(NT):
            r = pl.ds(i * TM, TM)
            pltpu.make_async_copy(out_v.at[r], out_hbm.at[r], osem.at[i]).wait()

    return kernel


def _build():
    TM, FC = 256, 512
    kern = make_kernel(TM, FC, False)
    NT = S // TM

    def f(A_x, A_wqkv, A_wo, B_w1, B_w3, B_w2, c, w_mod):
        x = A_x.reshape(S, D)
        anyspec = pl.BlockSpec(memory_space=pl.ANY)
        out = pl.pallas_call(
            kern,
            in_specs=[anyspec] * 8,
            out_specs=anyspec,
            out_shape=jax.ShapeDtypeStruct((S, D), bf16),
            scratch_shapes=[
                pltpu.VMEM((S, D), bf16),
                pltpu.VMEM((D, 3 * D), bf16),
                pltpu.VMEM((8, D, 128), bf16),
                pltpu.VMEM((D, D), bf16),
                pltpu.VMEM((D, F), bf16), pltpu.VMEM((D, F), bf16), pltpu.VMEM((F, D), bf16),
                pltpu.VMEM((1, D), bf16),
                pltpu.VMEM((D, 2 * D), bf16), pltpu.VMEM((D, D), bf16), pltpu.VMEM((D, 3 * D), bf16),
                pltpu.VMEM((8, 6 * D), f32),
                pltpu.VMEM((TM, D), bf16),
                pltpu.VMEM((16, HALO + TM, 128), f32),
                pltpu.VMEM((S, D), f32),
                pltpu.VMEM((S, D), bf16),
                pltpu.SemaphoreType.DMA((20,)),
                pltpu.SemaphoreType.DMA((NT,)),
            ],
            compiler_params=pltpu.CompilerParams(vmem_limit_bytes=120 * 2**20),
        )(x, A_wqkv, A_wo, B_w1, B_w3, B_w2, c, w_mod)
        return out.reshape(1, S, D)
    return f


@jax.jit
def pallas_adaLN_cond__sliding_local_dilated__glu_gated_swiglu__prompt_kernel(
    A_x: jax.Array,
    A_wqkv: jax.Array,
    A_wo: jax.Array,
    B_x: jax.Array,
    B_w1: jax.Array,
    B_w3: jax.Array,
    B_w2: jax.Array,
    c: jax.Array,
    w_mod: jax.Array,
):
    del B_x
    return _build()(A_x, A_wqkv, A_wo, B_w1, B_w3, B_w2, c, w_mod)
```

```python
import contextlib
import jax
import jax.numpy as jnp
from jax import lax
from jax.experimental import pallas as pl
from jax.experimental.pallas import tpu as pltpu

S, D, H, DH, F = 2048, 1024, 32, 32, 3584
W, DIL = 8, 2
HALO = 16
DT = D // 128
TM = 256
NT = S // TM
f32, bf16, i32 = jnp.float32, jnp.bfloat16, jnp.int32


def _normalize(xf):
    mean = jnp.sum(xf, axis=-1, keepdims=True) * (1.0 / D)
    xc = xf - mean
    var = jnp.sum(xc * xc, axis=-1, keepdims=True) * (1.0 / D)
    return xc * lax.rsqrt(var + 1e-5)


def _silu(g):
    hg = 0.5 * g
    return hg * jnp.tanh(hg) + hg


def _ld(wi):
    return jnp.concatenate([pltpu.bitcast(wi[j], bf16) for j in range(wi.shape[0])], axis=1)


def _st(dst, val, rows=slice(None)):
    for j in range(val.shape[1] // 128):
        dst[j, rows, :] = pltpu.bitcast(val[:, j * 128:(j + 1) * 128], i32)


def _or_all(vals):
    t = None
    for v in vals:
        v = pltpu.bitcast(v, i32)
        for r in range(0, v.shape[0], 8):
            t = v[r:r + 8] if t is None else t | v[r:r + 8]
    return t


def _xor_net(vs, masks):
    vs = list(vs)
    for b in range(3):
        nv = list(vs)
        for u in range(8):
            if not (u >> b) & 1:
                p = u | (1 << b)
                nv[u] = jnp.where(masks[b], vs[p], vs[u])
                nv[p] = jnp.where(masks[b], vs[u], vs[p])
        vs = nv
    return vs


def _permute_cols(wi, t0, G):
    R = 8 * G
    lane = lax.broadcasted_iota(i32, (R, 128), 1)
    masks = [((lane >> (2 + b)) & 1) == 1 for b in range(3)]
    r, j, a = lane >> 5, (lane >> 2) & 7, lane & 3
    idx = [a * 32 + (j ^ u) * 4 + r for u in range(8)]
    for g in range(0, wi.shape[1], R):
        rows = pl.ds(g, R)
        src = [wi[t0 + t, rows, :] for t in range(8)]
        mer = _xor_net(src, masks)
        per = [jnp.take_along_axis(mer[u], idx[u], axis=1) for u in range(8)]
        dst = _xor_net(per, masks)
        for t in range(8):
            wi[t0 + t, rows, :] = dst[t]


def _permute_rows(wi):
    sub = lax.broadcasted_iota(i32, (8, 128), 0)
    low = [((sub >> b) & 1) == 0 for b in range(3)]
    for j in range(DT):
        tgt = [None] * 64
        for eh in range(2):
            for mh in range(2):
                for par in range(2):
                    vs = []
                    for m in range(8 * mh, 8 * mh + 8):
                        A = wi[j, pl.ds((2 * m) * 16 + 8 * eh, 8), :]
                        B = wi[j, pl.ds((2 * m + 1) * 16 + 8 * eh, 8), :]
                        vs.append((A & 0xFFFF) | (B << 16) if par == 0
                                  else lax.shift_right_logical(A, 16) | (B & jnp.int32(-65536)))
                    for b in range(3):
                        s = 1 << b
                        nv = list(vs)
                        for u in range(8):
                            if not (u >> b) & 1:
                                p = u | s
                                nv[u] = jnp.where(low[b], vs[u], pltpu.roll(vs[p], s, 0))
                                nv[p] = jnp.where(low[b], pltpu.roll(vs[u], 8 - s, 0), vs[p])
                        vs = nv
                    for e in range(8):
                        tgt[(2 * (8 * eh + e) + par) * 2 + mh] = vs[e]
        wi[j] = jnp.concatenate(tgt, axis=0)


def _windows(full, M):
    outs = [None] * W
    for s in range(4):
        r = full if s == 0 else pltpu.roll(full, DIL * s, 0)
        outs[s] = r[HALO:HALO + M]
        outs[s + 4] = r[HALO - 8:HALO - 8 + M]
    return outs


def _softmax_weights(q, kfull, pos0):
    scale = DH ** -0.5
    pos = pos0 + lax.broadcasted_iota(i32, (TM, 128), 0)
    acc = [None] * W
    for j in range(DT):
        ks = _windows(kfull[j], TM)
        for w in range(W):
            p = q[j] * ks[w]
            acc[w] = p if acc[w] is None else acc[w] + p
    logits = []
    for w in range(W):
        a = acc[w]
        a = a + pltpu.roll(a, 64, 1)
        a = a + pltpu.roll(a, 32, 1)
        a = a * scale
        if w > 0:
            a = jnp.where(pos >= DIL * w, a, -1e9)
        logits.append(a)
    m = logits[0]
    for w in range(1, W):
        m = jnp.maximum(m, logits[w])
    es = [jnp.exp(l - m) for l in logits]
    den = es[0]
    for w in range(1, W):
        den = den + es[w]
    inv = 1.0 / den
    return [e * inv for e in es], inv


def _pv(ps, vfull, R=32):
    outs = []
    for r0 in range(0, TM, R):
        vs = _windows(vfull[r0:r0 + HALO + R], R)
        acc = None
        for w in range(W):
            p = ps[w][r0:r0 + R] * vs[w]
            acc = p if acc is None else acc + p
        outs.append(acc)
    return jnp.concatenate(outs, axis=0)


def make_kernel(cfg):
    FH = F // 2
    FC = cfg.get('FC', 1792)
    PG = cfg.get('PG', 8)
    scopes = cfg.get('scopes', False)
    TILED = cfg.get('TILED', True)

    def sc(name):
        return jax.named_scope(name) if scopes else contextlib.nullcontext()

    def kernel(x_hbm, wqkv_hbm, wo_hbm, w1_hbm, w3_hbm, w2_hbm, c_hbm, wmod_hbm, out_hbm,
               x_v, wqkv_v, wo_v, w1_v, w3_v, w2_v, c_v, wm_v, wmc_v,
               mod_v, modc_v, ct_v, h_i, o_i, halo_v, x1_v, h2_i, acc_v, out_v, sems, osem, msem, z_s):
        def cp(src, dst, k):
            return pltpu.make_async_copy(src, dst, sems.at[k])

        def tile_cps(src, dst, j0, j1, k):
            return [cp(src.at[:, j * 128:(j + 1) * 128], dst.at[j], k) for j in range(j0, j1)]

        def start(cs):
            for c_ in cs:
                c_.start()

        def wait(cs, name=None):
            with (sc(name) if name else contextlib.nullcontext()):
                for c_ in cs:
                    c_.wait()

        def wm_cp(p):
            return cp(wmod_hbm.at[:, pl.ds(pl.multiple_of(p * D, D), D)], wm_v.at[p], 12 + p)

        def wmc_cp(c):
            col = pl.multiple_of(3 * D + jnp.minimum(c, 5) * 512, 512)
            return pltpu.make_async_copy(wmod_hbm.at[:, pl.ds(col, 512)], wmc_v.at[c], msem.at[c])

        c_cp = cp(c_hbm, c_v, 0)
        x0_cp = cp(x_hbm.at[0:TM], x_v.at[0:TM], 1)
        x1_cp = cp(x_hbm.at[TM:2 * TM], x_v.at[TM:2 * TM], 2)
        x2_cp = cp(x_hbm.at[2 * TM:3 * TM], x_v.at[2 * TM:3 * TM], 10)
        x3_cp = cp(x_hbm.at[3 * TM:S], x_v.at[3 * TM:S], 11)
        wq_cps = tile_cps(wqkv_hbm, wqkv_v, 0, 8, 3)
        wk_cps = tile_cps(wqkv_hbm, wqkv_v, 8, 16, 4)
        wv_cps = tile_cps(wqkv_hbm, wqkv_v, 16, 24, 5)
        wo_cps = tile_cps(wo_hbm, wo_v, 0, 8, 6)
        if TILED:
            w1_cps = tile_cps(w1_hbm, w1_v, 0, F // 128, 7)
            w3_cps = tile_cps(w3_hbm, w3_v, 0, F // 128, 8)
            w2_cps = tile_cps(w2_hbm, w2_v, 0, DT, 9)
            w1_i, w3_i, w2_i = w1_v.bitcast(i32), w3_v.bitcast(i32), w2_v.bitcast(i32)
        else:
            w1_cps, w3_cps, w2_cps = [cp(w1_hbm, w1_v, 7)], [cp(w3_hbm, w3_v, 8)], [cp(w2_hbm, w2_v, 9)]

        start([c_cp, x0_cp] + wq_cps + [wm_cp(1), wm_cp(0)] + wk_cps + [x1_cp] + wv_cps + wo_cps + [wm_cp(2)])

        wqkv_i = wqkv_v.bitcast(i32)
        wo_i = wo_v.bitcast(i32)

        halo_v[...] = jnp.zeros((16, HALO, 128), f32)
        acc_v[...] = jnp.zeros_like(acc_v)
        z_s[0] = jnp.int32(0)

        c_cp.wait()
        cf = c_v[...].astype(f32)
        sf = (cf * jax.nn.sigmoid(cf)).astype(bf16)
        sc16 = jnp.broadcast_to(sf, (16, D))
        sf = sf.astype(f32)
        for t in range(DT):
            ct_v[t * 128:(t + 1) * 128, :] = jnp.broadcast_to(sf[:, t * 128:(t + 1) * 128], (128, 128)).T

        def zvec():
            return jnp.full((8, 128), z_s[0], i32)

        def ldw(wi, j, pin=None):
            w = wi[j]
            if pin is not None:
                w = jnp.concatenate([w[0:8] | (pltpu.bitcast(pin, i32) & zvec()), w[8:]], axis=0)
            return pltpu.bitcast(w, bf16)

        def mm(lhs, wi, j, pin=None):
            return jnp.dot(lhs, ldw(wi, j, pin), preferred_element_type=f32)

        def mod_fin(p, pins=None):
            if pins is None:
                r = jnp.dot(sc16, wm_v[p], preferred_element_type=f32)[0:8]
            else:
                wmi = wm_v.bitcast(i32)
                rs = []
                for n in range(DT):
                    w = wmi[p, :, n * 128:(n + 1) * 128]
                    w = jnp.concatenate([w[0:8] | (pins[n] & zvec()), w[8:]], axis=0)
                    rs.append(jnp.dot(sc16, pltpu.bitcast(w, bf16), preferred_element_type=f32)[0:8])
                r = jnp.concatenate(rs, axis=1)
            mod_v[p] = r + jnp.where(p == 1, 1.0, 0.0)

        def mod(k):
            if k >= 3:
                return jnp.concatenate([modc_v[(k - 3) * 8 + j, 0:1, :] for j in range(DT)], axis=1)
            return mod_v[k, 0:1, :]

        def ln1_val(t):
            r = pl.ds(pl.multiple_of(t * TM, TM), TM)
            return (_normalize(x_v[r, :].astype(f32)) * mod(1) + mod(0)).astype(bf16)

        def ln_pins(hv):
            rp = TM // 8
            return [_or_all([hv[n * rp:(n + 1) * rp, c * 128:(c + 1) * 128] for c in range(DT)]) for n in range(8)]

        def o_phase(t, pins):
            r = pl.ds(pl.multiple_of(t * TM, TM), TM)
            o = _ld(o_i)
            for n in range(DT):
                cs = slice(n * 128, (n + 1) * 128)
                y = mm(o, wo_i, n, pins[n])
                x1_v[r, cs] = x_v[r, cs].astype(f32) + mod_v[2, 0:1, cs] * y

        def kv_tile(h, sec, n, pin=None):
            y = mm(h, wqkv_i, 8 * sec + n, pin)
            full = jnp.concatenate([halo_v[8 * (sec - 1) + n], y], axis=0)
            halo_v[8 * (sec - 1) + n] = y[TM - HALO:]
            return full

        def mod_chunk(i):
            w = wmc_v[i - 1].astype(f32)
            outs = []
            for e in range(4):
                p = w[:, e * 128:(e + 1) * 128] * ct_v[...]
                acc = None
                for r in range(0, D, 8):
                    acc = p[r:r + 8] if acc is None else acc + p[r:r + 8]
                for s in (4, 2, 1):
                    acc = acc + pltpu.roll(acc, s, 0)
                outs.append(acc)
            d0 = jnp.minimum(i - 1, 5) * 4
            for e in range(4):
                tau = d0 + e
                modc_v[tau] = outs[e] + (tau // 8 == 1).astype(f32)
            return outs

        with sc('wq_perm'):
            wait(wq_cps)
            _permute_cols(wqkv_i, 0, PG)
        with sc('xhat0'):
            x0_cp.wait()
            x1_v[0:TM, :] = _normalize(x_v[0:TM, :].astype(f32))
        with sc('mod_a'):
            def mbody(t, carry):
                wm_cp(1 - t).wait()
                mod_fin(1 - t)
                return carry
            lax.fori_loop(0, 2, mbody, 0)

        with sc('A0'):
            _st(h_i, (x1_v[0:TM, :] * mod(1) + mod(0)).astype(bf16))
            h = _ld(h_i)
            q = []
            for n in range(8):
                if n == 4:
                    wait(wk_cps, 'w_wk')
                    _permute_cols(wqkv_i, 8, PG)
                q.append(mm(h, wqkv_i, n))
            wait([x1_cp], 'w_x1')
            hn = ln1_val(1)
            pins = ln_pins(hn)
            pins = [None, pins[0] | pins[1], pins[2] | pins[3] | pins[4], pins[5] | pins[6] | pins[7]] + [None] * 4
            kfull = []
            for n in range(8):
                if n == 4:
                    wait(wv_cps, 'w_wv')
                    _permute_cols(wqkv_i, 16, PG)
                kfull.append(kv_tile(h, 1, n, pins[n]))
            ps, inv = _softmax_weights(q, kfull, 0)
            vfull = []
            for n in range(8):
                pin = None
                if n >= 1:
                    lo, hi = (n - 1) * TM // 7 // 8 * 8, (TM if n == 7 else n * TM // 7 // 8 * 8)
                    pin = _or_all([inv[lo:hi]])
                vfull.append(kv_tile(h, 2, n, pin))
            wait(wo_cps, 'w_wo')
            wait([wm_cp(2)], 'w_wm2')
            start([x2_cp, wmc_cp(0), x3_cp])
            _permute_rows(wo_i)
            of = [_pv(ps, vfull[j]) for j in range(DT)]
            mod_fin(2, [_or_all([of[n]]) for n in range(DT)])
            _st(o_i, jnp.concatenate([o_.astype(bf16) for o_ in of], axis=1))
            _st(h_i, hn)

        def a_body(i):
            h = _ld(h_i)
            mouts = mod_chunk(i)
            q = [mm(h, wqkv_i, n, mouts[n - 2] if 2 <= n < 6 else None) for n in range(8)]
            hn = ln1_val(jnp.minimum(i + 1, NT - 1))
            pins = ln_pins(hn)
            kfull = [kv_tile(h, 1, n, pins[n]) for n in range(8)]
            ps, inv = _softmax_weights(q, kfull, i * TM)
            vfull = [kv_tile(h, 2, n) for n in range(8)]
            of = [_pv(ps, vfull[j]) for j in range(DT)]
            o_phase(i - 1, [_or_all([of[n]]) for n in range(DT)])
            _st(o_i, jnp.concatenate([o_.astype(bf16) for o_ in of], axis=1))
            _st(h_i, hn)

        def a_loop(i, carry):
            wmc_cp(i - 1).wait()
            for it_, waits, starts in ((1, [x2_cp], [wmc_cp(c) for c in range(1, 7)]),
                                       (2, [x3_cp], w1_cps), (4, [], w3_cps), (6, [], w2_cps)):
                @pl.when(i == it_)
                def _(waits=waits, starts=starts):
                    wait(waits)
                    start(starts)

            with sc('Ait'):
                a_body(i)
            return carry
        lax.fori_loop(1, NT, a_loop, 0)

        with sc('wo7'):
            wait(w1_cps + w3_cps + w2_cps)
            h20 = (_normalize(x1_v[0:TM, :]) * mod(4) + mod(3)).astype(bf16)
            o_phase(NT - 1, ln_pins(h20))
            _st(h2_i.at[0], h20)

        def f_iter(it):
            i = it // 2
            half = it % 2
            r = pl.ds(pl.multiple_of(i * TM, TM), TM)
            h2 = _ld(h2_i.at[i % 2])
            hm = TM // 2
            t = jnp.minimum(i + 1, NT - 1)
            rr = pl.ds(pl.multiple_of(t * TM + half * hm, hm), hm)
            hn = (_normalize(x1_v[rr, :]) * mod(4) + mod(3)).astype(bf16)
            acc = acc_v[...] * half.astype(f32)
            c0 = pl.multiple_of(half * FH, FH)
            for c in range(FH // FC):
                if TILED:
                    t0 = half * (FH // 128) + c * (FC // 128)
                    lt = lambda wi: jnp.concatenate([pltpu.bitcast(wi[t0 + e], bf16) for e in range(FC // 128)], axis=1)
                    g = jnp.dot(h2, lt(w1_i), preferred_element_type=f32)
                    u = jnp.dot(h2, lt(w3_i), preferred_element_type=f32)
                    a = (_silu(g) * u).astype(bf16)
                    kr = pl.ds(pl.multiple_of(t0 * 64, 64), FC // 2)
                    w2 = jnp.concatenate([pltpu.bitcast(w2_i[j, kr, :], bf16) for j in range(DT)], axis=1)
                    acc = acc + jnp.dot(a, w2, preferred_element_type=f32)
                    continue
                cs = pl.ds(c0 + c * FC, FC)
                g = jnp.dot(h2, w1_v[:, cs], preferred_element_type=f32)
                u = jnp.dot(h2, w3_v[:, cs], preferred_element_type=f32)
                a = (_silu(g) * u).astype(bf16)
                acc = acc + jnp.dot(a, w2_v[cs, :], preferred_element_type=f32)
            acc_v[...] = acc
            out_v[r, :] = (x1_v[r, :] + mod(5) * acc).astype(out_v.dtype)
            _st(h2_i.at[(i + 1) % 2], hn, rows=pl.ds(pl.multiple_of(half * (hm // 2), hm // 2), hm // 2))

            @pl.when(half == 1)
            def _():
                pltpu.make_async_copy(out_v.at[r], out_hbm.at[r], osem.at[i]).start()

        def f_loop(it, carry):
            with sc('Fit'):
                f_iter(it)
            return carry
        lax.fori_loop(0, 2 * NT, f_loop, 0)
        with sc('tail'):
            for i in range(NT):
                r = pl.ds(i * TM, TM)
                pltpu.make_async_copy(out_v.at[r], out_hbm.at[r], osem.at[i]).wait()

    return kernel


def build(debug=False, **cfg):
    kern = make_kernel(cfg)
    odt = f32 if debug else bf16

    def f(A_x, A_wqkv, A_wo, B_w1, B_w3, B_w2, c, w_mod):
        x = A_x.reshape(S, D)
        anyspec = pl.BlockSpec(memory_space=pl.ANY)
        out = pl.pallas_call(
            kern,
            in_specs=[anyspec] * 8,
            out_specs=anyspec,
            out_shape=jax.ShapeDtypeStruct((S, D), odt),
            scratch_shapes=[
                pltpu.VMEM((S, D), bf16),
                pltpu.VMEM((3 * DT, D, 128), bf16),
                pltpu.VMEM((DT, D, 128), bf16),
                *([pltpu.VMEM((F // 128, D, 128), bf16), pltpu.VMEM((F // 128, D, 128), bf16), pltpu.VMEM((DT, F, 128), bf16)] if cfg.get('TILED', True)
                  else [pltpu.VMEM((D, F), bf16), pltpu.VMEM((D, F), bf16), pltpu.VMEM((F, D), bf16)]),
                pltpu.VMEM((1, D), bf16),
                pltpu.VMEM((3, D, D), bf16),
                pltpu.VMEM((7, D, 512), bf16),
                pltpu.VMEM((3, 8, D), f32),
                pltpu.VMEM((24, 8, 128), f32),
                pltpu.VMEM((D, 128), f32),
                pltpu.VMEM((DT, TM // 2, 128), i32),
                pltpu.VMEM((DT, TM // 2, 128), i32),
                pltpu.VMEM((16, HALO, 128), f32),
                pltpu.VMEM((S, D), f32),
                pltpu.VMEM((2, DT, TM // 2, 128), i32),
                pltpu.VMEM((TM, D), f32),
                pltpu.VMEM((S, D), odt),
                pltpu.SemaphoreType.DMA((16,)),
                pltpu.SemaphoreType.DMA((NT,)),
                pltpu.SemaphoreType.DMA((7,)),
                pltpu.SMEM((1,), i32),
            ],
            compiler_params=pltpu.CompilerParams(vmem_limit_bytes=120 * 2**20),
        )(x, A_wqkv, A_wo, B_w1, B_w3, B_w2, c, w_mod)
        return out.reshape(1, S, D)
    return f


@jax.jit
def pallas_adaLN_cond__sliding_local_dilated__glu_gated_swiglu__prompt_kernel(
    A_x: jax.Array,
    A_wqkv: jax.Array,
    A_wo: jax.Array,
    B_x: jax.Array,
    B_w1: jax.Array,
    B_w3: jax.Array,
    B_w2: jax.Array,
    c: jax.Array,
    w_mod: jax.Array,
):
    del B_x
    return build()(A_x, A_wqkv, A_wo, B_w1, B_w3, B_w2, c, w_mod)
```

```python
import contextlib
import jax
import jax.numpy as jnp
from jax import lax
from jax.experimental import pallas as pl
from jax.experimental.pallas import tpu as pltpu

S, D, H, DH, F = 2048, 1024, 32, 32, 3584
W, DIL = 8, 2
HALO = 16
DT = D // 128
TM = 256
NT = S // TM
f32, bf16, i32 = jnp.float32, jnp.bfloat16, jnp.int32


def _normalize(xf):
    mean = jnp.sum(xf, axis=-1, keepdims=True) * (1.0 / D)
    xc = xf - mean
    var = jnp.sum(xc * xc, axis=-1, keepdims=True) * (1.0 / D)
    return xc * lax.rsqrt(var + 1e-5)


def _silu(g):
    hg = 0.5 * g
    return hg * jnp.tanh(hg) + hg


def _ld(wi):
    return jnp.concatenate([pltpu.bitcast(wi[j], bf16) for j in range(wi.shape[0])], axis=1)


def _st(dst, val, rows=slice(None)):
    for j in range(val.shape[1] // 128):
        dst[j, rows, :] = pltpu.bitcast(val[:, j * 128:(j + 1) * 128], i32)


def _pack(val):
    return [pltpu.bitcast(val[:, j * 128:(j + 1) * 128], i32) for j in range(val.shape[1] // 128)]


def _or_all(vals):
    t = None
    for v in vals:
        v = pltpu.bitcast(v, i32)
        for r in range(0, v.shape[0], 8):
            t = v[r:r + 8] if t is None else t | v[r:r + 8]
    return t


def _xor_net(vs, masks):
    vs = list(vs)
    for b in range(3):
        nv = list(vs)
        for u in range(8):
            if not (u >> b) & 1:
                p = u | (1 << b)
                nv[u] = jnp.where(masks[b], vs[p], vs[u])
                nv[p] = jnp.where(masks[b], vs[u], vs[p])
        vs = nv
    return vs


def _permute_cols(wi, t0, G):
    R = 8 * G
    lane = lax.broadcasted_iota(i32, (R, 128), 1)
    masks = [((lane >> (2 + b)) & 1) == 1 for b in range(3)]
    r, j, a = lane >> 5, (lane >> 2) & 7, lane & 3
    idx = [a * 32 + (j ^ u) * 4 + r for u in range(8)]
    for g in range(0, wi.shape[1], R):
        rows = pl.ds(g, R)
        src = [wi[t0 + t, rows, :] for t in range(8)]
        mer = _xor_net(src, masks)
        per = [jnp.take_along_axis(mer[u], idx[u], axis=1) for u in range(8)]
        dst = _xor_net(per, masks)
        for t in range(8):
            wi[t0 + t, rows, :] = dst[t]


def _permute_rows(wi):
    sub = lax.broadcasted_iota(i32, (8, 128), 0)
    low = [((sub >> b) & 1) == 0 for b in range(3)]
    for j in range(DT):
        tgt = [None] * 64
        for eh in range(2):
            for mh in range(2):
                for par in range(2):
                    vs = []
                    for m in range(8 * mh, 8 * mh + 8):
                        A = wi[j, pl.ds((2 * m) * 16 + 8 * eh, 8), :]
                        B = wi[j, pl.ds((2 * m + 1) * 16 + 8 * eh, 8), :]
                        vs.append((A & 0xFFFF) | (B << 16) if par == 0
                                  else lax.shift_right_logical(A, 16) | (B & jnp.int32(-65536)))
                    for b in range(3):
                        s = 1 << b
                        nv = list(vs)
                        for u in range(8):
                            if not (u >> b) & 1:
                                p = u | s
                                nv[u] = jnp.where(low[b], vs[u], pltpu.roll(vs[p], s, 0))
                                nv[p] = jnp.where(low[b], pltpu.roll(vs[u], 8 - s, 0), vs[p])
                        vs = nv
                    for e in range(8):
                        tgt[(2 * (8 * eh + e) + par) * 2 + mh] = vs[e]
        wi[j] = jnp.concatenate(tgt, axis=0)


def _windows(full, M):
    outs = [None] * W
    for s in range(4):
        r = full if s == 0 else pltpu.roll(full, DIL * s, 0)
        outs[s] = r[HALO:HALO + M]
        outs[s + 4] = r[HALO - 8:HALO - 8 + M]
    return outs


def _softmax_weights(q, kfull, pos0):
    scale = DH ** -0.5
    pos = pos0 + lax.broadcasted_iota(i32, (TM, 128), 0)
    acc = [None] * W
    for j in range(DT):
        ks = _windows(kfull[j], TM)
        for w in range(W):
            p = q[j] * ks[w]
            acc[w] = p if acc[w] is None else acc[w] + p
    logits = []
    for w in range(W):
        a = acc[w]
        a = a + pltpu.roll(a, 64, 1)
        a = a + pltpu.roll(a, 32, 1)
        a = a * scale
        if w > 0:
            a = jnp.where(pos >= DIL * w, a, -1e9)
        logits.append(a)
    m = logits[0]
    for w in range(1, W):
        m = jnp.maximum(m, logits[w])
    es = [jnp.exp(l - m) for l in logits]
    den = es[0]
    for w in range(1, W):
        den = den + es[w]
    inv = 1.0 / den
    return [e * inv for e in es], inv


def _pv(ps, vfull, R=32):
    outs = []
    for r0 in range(0, TM, R):
        vs = _windows(vfull[r0:r0 + HALO + R], R)
        acc = None
        for w in range(W):
            p = ps[w][r0:r0 + R] * vs[w]
            acc = p if acc is None else acc + p
        outs.append(acc)
    return jnp.concatenate(outs, axis=0)


def make_kernel(cfg):
    FH = F // 2
    FC = cfg.get('FC', 1792)
    PG = cfg.get('PG', 8)
    scopes = cfg.get('scopes', False)
    TILED = cfg.get('TILED', True)
    FPIN = cfg.get('FPIN', True)
    FP0 = cfg.get('FP0', 2)
    FPS = cfg.get('FPS', 1)

    def sc(name):
        return jax.named_scope(name) if scopes else contextlib.nullcontext()

    def kernel(x_hbm, wqkv_hbm, wo_hbm, w1_hbm, w3_hbm, w2_hbm, c_hbm, wmod_hbm, out_hbm,
               x_v, wqkv_v, wo_v, w1_v, w3_v, w2_v, c_v, wm_v, wmc_v,
               mod_v, modc_v, ct_v, h_i, o_i, halo_v, x1_v, h2_i, acc_v, out_v, sems, osem, msem, z_s):
        def cp(src, dst, k):
            return pltpu.make_async_copy(src, dst, sems.at[k])

        def tile_cps(src, dst, j0, j1, k):
            return [cp(src.at[:, j * 128:(j + 1) * 128], dst.at[j], k) for j in range(j0, j1)]

        def start(cs):
            for c_ in cs:
                c_.start()

        def wait(cs, name=None):
            with (sc(name) if name else contextlib.nullcontext()):
                for c_ in cs:
                    c_.wait()

        def wm_cp(p):
            return cp(wmod_hbm.at[:, pl.ds(pl.multiple_of(p * D, D), D)], wm_v.at[p], 12 + p)

        def wmc_cp(c):
            col = pl.multiple_of(3 * D + jnp.minimum(c, 5) * 512, 512)
            return pltpu.make_async_copy(wmod_hbm.at[:, pl.ds(col, 512)], wmc_v.at[c], msem.at[c])

        c_cp = cp(c_hbm, c_v, 0)
        x0_cp = cp(x_hbm.at[0:TM], x_v.at[0:TM], 1)
        x1_cp = cp(x_hbm.at[TM:2 * TM], x_v.at[TM:2 * TM], 2)
        x2_cp = cp(x_hbm.at[2 * TM:3 * TM], x_v.at[2 * TM:3 * TM], 10)
        x3_cp = cp(x_hbm.at[3 * TM:S], x_v.at[3 * TM:S], 11)
        wq_cps = tile_cps(wqkv_hbm, wqkv_v, 0, 8, 3)
        wk_cps = tile_cps(wqkv_hbm, wqkv_v, 8, 16, 4)
        wv_cps = tile_cps(wqkv_hbm, wqkv_v, 16, 24, 5)
        wo_cps = tile_cps(wo_hbm, wo_v, 0, 8, 6)
        if TILED:
            w1_cps = tile_cps(w1_hbm, w1_v, 0, F // 128, 7)
            w3_cps = tile_cps(w3_hbm, w3_v, 0, F // 128, 8)
            w2_cps = tile_cps(w2_hbm, w2_v, 0, DT, 9)
            w1_i, w3_i, w2_i = w1_v.bitcast(i32), w3_v.bitcast(i32), w2_v.bitcast(i32)
        else:
            w1_cps, w3_cps, w2_cps = [cp(w1_hbm, w1_v, 7)], [cp(w3_hbm, w3_v, 8)], [cp(w2_hbm, w2_v, 9)]

        start([c_cp, x0_cp] + wq_cps + [wm_cp(1), wm_cp(0)] + wk_cps + [x1_cp] + wv_cps + wo_cps + [wm_cp(2)])

        wqkv_i = wqkv_v.bitcast(i32)
        wo_i = wo_v.bitcast(i32)

        halo_v[...] = jnp.zeros((16, HALO, 128), f32)
        acc_v[...] = jnp.zeros_like(acc_v)
        z_s[0] = jnp.int32(0)

        c_cp.wait()
        cf = c_v[...].astype(f32)
        sf = (cf * jax.nn.sigmoid(cf)).astype(bf16)
        sc16 = jnp.broadcast_to(sf, (16, D))
        sf = sf.astype(f32)
        for t in range(DT):
            ct_v[t * 128:(t + 1) * 128, :] = jnp.broadcast_to(sf[:, t * 128:(t + 1) * 128], (128, 128)).T

        def zvec():
            return jnp.full((8, 128), z_s[0], i32)

        def ldw(wi, j, pin=None):
            w = wi[j]
            if pin is not None:
                w = jnp.concatenate([w[0:8] | (pltpu.bitcast(pin, i32) & zvec()), w[8:]], axis=0)
            return pltpu.bitcast(w, bf16)

        def mm(lhs, wi, j, pin=None):
            return jnp.dot(lhs, ldw(wi, j, pin), preferred_element_type=f32)

        def mod_fin(p, pins=None):
            if pins is None:
                r = jnp.dot(sc16, wm_v[p], preferred_element_type=f32)[0:8]
            else:
                wmi = wm_v.bitcast(i32)
                rs = []
                for n in range(DT):
                    w = wmi[p, :, n * 128:(n + 1) * 128]
                    w = jnp.concatenate([w[0:8] | (pins[n] & zvec()), w[8:]], axis=0)
                    rs.append(jnp.dot(sc16, pltpu.bitcast(w, bf16), preferred_element_type=f32)[0:8])
                r = jnp.concatenate(rs, axis=1)
            mod_v[p] = r + jnp.where(p == 1, 1.0, 0.0)

        def mod(k):
            if k >= 3:
                return jnp.concatenate([modc_v[(k - 3) * 8 + j, 0:1, :] for j in range(DT)], axis=1)
            return mod_v[k, 0:1, :]

        def ln1_val(t):
            r = pl.ds(pl.multiple_of(t * TM, TM), TM)
            return _pack((_normalize(x_v[r, :].astype(f32)) * mod(1) + mod(0)).astype(bf16))

        def ln_pins(hw):
            rp = hw[0].shape[0] // 8
            return [_or_all([t[n * rp:(n + 1) * rp] for t in hw]) for n in range(8)]

        def st_tiles(dst, tiles, rows=slice(None)):
            for j, t in enumerate(tiles):
                dst[j, rows, :] = t

        def o_phase(t, pins):
            r = pl.ds(pl.multiple_of(t * TM, TM), TM)
            o = _ld(o_i)
            for n in range(DT):
                cs = slice(n * 128, (n + 1) * 128)
                y = mm(o, wo_i, n, pins[n])
                x1_v[r, cs] = x_v[r, cs].astype(f32) + mod_v[2, 0:1, cs] * y

        def kv_tile(h, sec, n, pin=None):
            y = mm(h, wqkv_i, 8 * sec + n, pin)
            full = jnp.concatenate([halo_v[8 * (sec - 1) + n], y], axis=0)
            halo_v[8 * (sec - 1) + n] = y[TM - HALO:]
            return full

        def mod_chunk(i):
            w = wmc_v[i - 1].astype(f32)
            outs = []
            for e in range(4):
                p = w[:, e * 128:(e + 1) * 128] * ct_v[...]
                acc = None
                for r in range(0, D, 8):
                    acc = p[r:r + 8] if acc is None else acc + p[r:r + 8]
                for s in (4, 2, 1):
                    acc = acc + pltpu.roll(acc, s, 0)
                outs.append(acc)
            d0 = jnp.minimum(i - 1, 5) * 4
            for e in range(4):
                tau = d0 + e
                modc_v[tau] = outs[e] + (tau // 8 == 1).astype(f32)
            return outs

        with sc('wq_perm'):
            wait(wq_cps)
            _permute_cols(wqkv_i, 0, PG)
        with sc('xhat0'):
            x0_cp.wait()
            x1_v[0:TM, :] = _normalize(x_v[0:TM, :].astype(f32))
        with sc('mod_a'):
            def mbody(t, carry):
                wm_cp(1 - t).wait()
                mod_fin(1 - t)
                return carry
            lax.fori_loop(0, 2, mbody, 0)

        with sc('A0'):
            _st(h_i, (x1_v[0:TM, :] * mod(1) + mod(0)).astype(bf16))
            h = _ld(h_i)
            q = []
            for n in range(8):
                if n == 4:
                    wait(wk_cps, 'w_wk')
                    _permute_cols(wqkv_i, 8, PG)
                q.append(mm(h, wqkv_i, n))
            wait([x1_cp], 'w_x1')
            hn = ln1_val(1)
            pins = ln_pins(hn)
            pins = [None, pins[0] | pins[1], pins[2] | pins[3] | pins[4], pins[5] | pins[6] | pins[7]] + [None] * 4
            kfull = []
            for n in range(8):
                if n == 4:
                    wait(wv_cps, 'w_wv')
                    _permute_cols(wqkv_i, 16, PG)
                kfull.append(kv_tile(h, 1, n, pins[n]))
            ps, inv = _softmax_weights(q, kfull, 0)
            vfull = []
            for n in range(8):
                pin = None
                if n >= 1:
                    lo, hi = (n - 1) * TM // 7 // 8 * 8, (TM if n == 7 else n * TM // 7 // 8 * 8)
                    pin = _or_all([inv[lo:hi]])
                vfull.append(kv_tile(h, 2, n, pin))
            wait(wo_cps, 'w_wo')
            wait([wm_cp(2)], 'w_wm2')
            start([x2_cp, wmc_cp(0), x3_cp])
            _permute_rows(wo_i)
            of = [_pv(ps, vfull[j]) for j in range(DT)]
            mod_fin(2, [_or_all([of[n]]) for n in range(DT)])
            _st(o_i, jnp.concatenate([o_.astype(bf16) for o_ in of], axis=1))
            st_tiles(h_i, hn)

        def a_body(i):
            h = _ld(h_i)
            mouts = mod_chunk(i)
            q = [mm(h, wqkv_i, n, mouts[n - 2] if 2 <= n < 6 else None) for n in range(8)]
            hn = ln1_val(jnp.minimum(i + 1, NT - 1))
            pins = ln_pins(hn)
            kfull = [kv_tile(h, 1, n, pins[n]) for n in range(8)]
            ps, inv = _softmax_weights(q, kfull, i * TM)
            vfull = [kv_tile(h, 2, n) for n in range(8)]
            of = [_pv(ps, vfull[j]) for j in range(DT)]
            o_phase(i - 1, [_or_all([of[n]]) for n in range(DT)])
            _st(o_i, jnp.concatenate([o_.astype(bf16) for o_ in of], axis=1))
            st_tiles(h_i, hn)

        def a_loop(i, carry):
            wmc_cp(i - 1).wait()
            for it_, waits, starts in ((1, [x2_cp], [wmc_cp(c) for c in range(1, 7)]),
                                       (2, [x3_cp], w1_cps), (4, [], w3_cps), (6, [], w2_cps)):
                @pl.when(i == it_)
                def _(waits=waits, starts=starts):
                    wait(waits)
                    start(starts)

            with sc('Ait'):
                a_body(i)
            return carry
        lax.fori_loop(1, NT, a_loop, 0)

        with sc('wo7'):
            wait(w1_cps + w3_cps + w2_cps)
            h20 = _pack((_normalize(x1_v[0:TM, :]) * mod(4) + mod(3)).astype(bf16))
            o_phase(NT - 1, ln_pins(h20))
            st_tiles(h2_i.at[0], h20)

        def f_iter(it):
            i = it // 2
            half = it % 2
            r = pl.ds(pl.multiple_of(i * TM, TM), TM)
            h2 = _ld(h2_i.at[i % 2])
            hm = TM // 2
            t = jnp.minimum(i + 1, NT - 1)
            rr = pl.ds(pl.multiple_of(t * TM + half * hm, hm), hm)
            hn = _pack((_normalize(x1_v[rr, :]) * mod(4) + mod(3)).astype(bf16))
            pins = ln_pins(hn)
            acc = acc_v[...] * half.astype(f32)
            c0 = pl.multiple_of(half * FH, FH)
            for c in range(FH // FC):
                if TILED:
                    t0 = half * (FH // 128) + c * (FC // 128)
                    nt_ = FC // 128

                    def lt(wi, pp):
                        tiles = []
                        for e in range(nt_):
                            w = wi[t0 + e]
                            if pp is not None and pp.get(e) is not None:
                                w = jnp.concatenate([w[0:8] | (pp[e] & zvec()), w[8:]], axis=0)
                            tiles.append(pltpu.bitcast(w, bf16))
                        return jnp.concatenate(tiles, axis=1)
                    pp = {FP0 + n * FPS: pins[n] for n in range(8)} if (FPIN and c == 0) else None
                    g = jnp.dot(h2, lt(w1_i, pp), preferred_element_type=f32)
                    u = jnp.dot(h2, lt(w3_i, None), preferred_element_type=f32)
                    a = (_silu(g) * u).astype(bf16)
                    kr = pl.ds(pl.multiple_of(t0 * 64, 64), FC // 2)
                    w2 = jnp.concatenate([pltpu.bitcast(w2_i[j, kr, :], bf16) for j in range(DT)], axis=1)
                    acc = acc + jnp.dot(a, w2, preferred_element_type=f32)
                    continue
                cs = pl.ds(c0 + c * FC, FC)
                g = jnp.dot(h2, w1_v[:, cs], preferred_element_type=f32)
                u = jnp.dot(h2, w3_v[:, cs], preferred_element_type=f32)
                a = (_silu(g) * u).astype(bf16)
                acc = acc + jnp.dot(a, w2_v[cs, :], preferred_element_type=f32)
            acc_v[...] = acc
            out_v[r, :] = (x1_v[r, :] + mod(5) * acc).astype(out_v.dtype)
            st_tiles(h2_i.at[(i + 1) % 2], hn, rows=pl.ds(pl.multiple_of(half * (hm // 2), hm // 2), hm // 2))

            @pl.when(half == 1)
            def _():
                pltpu.make_async_copy(out_v.at[r], out_hbm.at[r], osem.at[i]).start()

        def f_loop(it, carry):
            with sc('Fit'):
                f_iter(it)
            return carry
        lax.fori_loop(0, 2 * NT, f_loop, 0)
        with sc('tail'):
            for i in range(NT):
                r = pl.ds(i * TM, TM)
                pltpu.make_async_copy(out_v.at[r], out_hbm.at[r], osem.at[i]).wait()

    return kernel


def build(debug=False, **cfg):
    kern = make_kernel(cfg)
    odt = f32 if debug else bf16

    def f(A_x, A_wqkv, A_wo, B_w1, B_w3, B_w2, c, w_mod):
        x = A_x.reshape(S, D)
        anyspec = pl.BlockSpec(memory_space=pl.ANY)
        out = pl.pallas_call(
            kern,
            in_specs=[anyspec] * 8,
            out_specs=anyspec,
            out_shape=jax.ShapeDtypeStruct((S, D), odt),
            scratch_shapes=[
                pltpu.VMEM((S, D), bf16),
                pltpu.VMEM((3 * DT, D, 128), bf16),
                pltpu.VMEM((DT, D, 128), bf16),
                *([pltpu.VMEM((F // 128, D, 128), bf16), pltpu.VMEM((F // 128, D, 128), bf16), pltpu.VMEM((DT, F, 128), bf16)] if cfg.get('TILED', True)
                  else [pltpu.VMEM((D, F), bf16), pltpu.VMEM((D, F), bf16), pltpu.VMEM((F, D), bf16)]),
                pltpu.VMEM((1, D), bf16),
                pltpu.VMEM((3, D, D), bf16),
                pltpu.VMEM((7, D, 512), bf16),
                pltpu.VMEM((3, 8, D), f32),
                pltpu.VMEM((24, 8, 128), f32),
                pltpu.VMEM((D, 128), f32),
                pltpu.VMEM((DT, TM // 2, 128), i32),
                pltpu.VMEM((DT, TM // 2, 128), i32),
                pltpu.VMEM((16, HALO, 128), f32),
                pltpu.VMEM((S, D), f32),
                pltpu.VMEM((2, DT, TM // 2, 128), i32),
                pltpu.VMEM((TM, D), f32),
                pltpu.VMEM((S, D), odt),
                pltpu.SemaphoreType.DMA((16,)),
                pltpu.SemaphoreType.DMA((NT,)),
                pltpu.SemaphoreType.DMA((7,)),
                pltpu.SMEM((1,), i32),
            ],
            compiler_params=pltpu.CompilerParams(vmem_limit_bytes=120 * 2**20),
        )(x, A_wqkv, A_wo, B_w1, B_w3, B_w2, c, w_mod)
        return out.reshape(1, S, D)
    return f


@jax.jit
def pallas_adaLN_cond__sliding_local_dilated__glu_gated_swiglu__prompt_kernel(
    A_x: jax.Array,
    A_wqkv: jax.Array,
    A_wo: jax.Array,
    B_x: jax.Array,
    B_w1: jax.Array,
    B_w3: jax.Array,
    B_w2: jax.Array,
    c: jax.Array,
    w_mod: jax.Array,
):
    del B_x
    return build()(A_x, A_wqkv, A_wo, B_w1, B_w3, B_w2, c, w_mod)
```

```python
import contextlib
import jax
import jax.numpy as jnp
from jax import lax
from jax.experimental import pallas as pl
from jax.experimental.pallas import tpu as pltpu

S, D, H, DH, F = 2048, 1024, 32, 32, 3584
W, DIL = 8, 2
HALO = 16
DT = D // 128
TM = 256
NT = S // TM
f32, bf16, i32 = jnp.float32, jnp.bfloat16, jnp.int32


def _normalize(xf):
    mean = jnp.sum(xf, axis=-1, keepdims=True) * (1.0 / D)
    xc = xf - mean
    var = jnp.sum(xc * xc, axis=-1, keepdims=True) * (1.0 / D)
    return xc * lax.rsqrt(var + 1e-5)


def _silu(g):
    hg = 0.5 * g
    return hg * jnp.tanh(hg) + hg


def _ld(wi):
    return jnp.concatenate([pltpu.bitcast(wi[j], bf16) for j in range(wi.shape[0])], axis=1)


def _st(dst, val, rows=slice(None)):
    for j in range(val.shape[1] // 128):
        dst[j, rows, :] = pltpu.bitcast(val[:, j * 128:(j + 1) * 128], i32)


def _pack(val):
    return [pltpu.bitcast(val[:, j * 128:(j + 1) * 128], i32) for j in range(val.shape[1] // 128)]


def _or_all(vals):
    t = None
    for v in vals:
        v = pltpu.bitcast(v, i32)
        for r in range(0, v.shape[0], 8):
            t = v[r:r + 8] if t is None else t | v[r:r + 8]
    return t


def _xor_net(vs, masks):
    vs = list(vs)
    for b in range(3):
        nv = list(vs)
        for u in range(8):
            if not (u >> b) & 1:
                p = u | (1 << b)
                nv[u] = jnp.where(masks[b], vs[p], vs[u])
                nv[p] = jnp.where(masks[b], vs[u], vs[p])
        vs = nv
    return vs


def _permute_cols(wi, t0, G, g0=0, g1=512):
    R = 8 * G
    lane = lax.broadcasted_iota(i32, (R, 128), 1)
    masks = [((lane >> (2 + b)) & 1) == 1 for b in range(3)]
    r, j, a = lane >> 5, (lane >> 2) & 7, lane & 3
    idx = [a * 32 + (j ^ u) * 4 + r for u in range(8)]
    for g in range(g0, g1, R):
        rows = pl.ds(g, R)
        src = [wi[t0 + t, rows, :] for t in range(8)]
        mer = _xor_net(src, masks)
        per = [jnp.take_along_axis(mer[u], idx[u], axis=1) for u in range(8)]
        dst = _xor_net(per, masks)
        for t in range(8):
            wi[t0 + t, rows, :] = dst[t]


def _permute_rows(wi):
    sub = lax.broadcasted_iota(i32, (8, 128), 0)
    low = [((sub >> b) & 1) == 0 for b in range(3)]
    done = []
    for j in range(DT):
        tgt = [None] * 64
        for eh in range(2):
            for mh in range(2):
                for par in range(2):
                    vs = []
                    for m in range(8 * mh, 8 * mh + 8):
                        A = wi[j, pl.ds((2 * m) * 16 + 8 * eh, 8), :]
                        B = wi[j, pl.ds((2 * m + 1) * 16 + 8 * eh, 8), :]
                        vs.append((A & 0xFFFF) | (B << 16) if par == 0
                                  else lax.shift_right_logical(A, 16) | (B & jnp.int32(-65536)))
                    for b in range(3):
                        s = 1 << b
                        nv = list(vs)
                        for u in range(8):
                            if not (u >> b) & 1:
                                p = u | s
                                nv[u] = jnp.where(low[b], vs[u], pltpu.roll(vs[p], s, 0))
                                nv[p] = jnp.where(low[b], pltpu.roll(vs[u], 8 - s, 0), vs[p])
                        vs = nv
                    for e in range(8):
                        tgt[(2 * (8 * eh + e) + par) * 2 + mh] = vs[e]
        wi[j] = jnp.concatenate(tgt, axis=0)
        done.append(tgt[63])
    return done


def _windows(full, M):
    outs = [None] * W
    for s in range(4):
        r = full if s == 0 else pltpu.roll(full, DIL * s, 0)
        outs[s] = r[HALO:HALO + M]
        outs[s + 4] = r[HALO - 8:HALO - 8 + M]
    return outs


def _softmax_weights(q, kfull, pos0):
    scale = DH ** -0.5
    pos = pos0 + lax.broadcasted_iota(i32, (TM, 128), 0)
    acc = [None] * W
    for j in range(DT):
        ks = _windows(kfull[j], TM)
        for w in range(W):
            p = q[j] * ks[w]
            acc[w] = p if acc[w] is None else acc[w] + p
    logits = []
    for w in range(W):
        a = acc[w]
        a = a + pltpu.roll(a, 64, 1)
        a = a + pltpu.roll(a, 32, 1)
        a = a * scale
        if w > 0:
            a = jnp.where(pos >= DIL * w, a, -1e9)
        logits.append(a)
    m = logits[0]
    for w in range(1, W):
        m = jnp.maximum(m, logits[w])
    es = [jnp.exp(l - m) for l in logits]
    den = es[0]
    for w in range(1, W):
        den = den + es[w]
    inv = 1.0 / den
    return [e * inv for e in es], inv


def _pv(ps, vfull, R=32):
    outs = []
    for r0 in range(0, TM, R):
        vs = _windows(vfull[r0:r0 + HALO + R], R)
        acc = None
        for w in range(W):
            p = ps[w][r0:r0 + R] * vs[w]
            acc = p if acc is None else acc + p
        outs.append(acc)
    return jnp.concatenate(outs, axis=0)


def make_kernel(cfg):
    FH = F // 2
    FC = cfg.get('FC', 1792)
    PG = cfg.get('PG', 8)
    scopes = cfg.get('scopes', False)
    TILED = cfg.get('TILED', True)
    QA, QB, KA, KB = cfg.get('QA', 2), cfg.get('QB', 6), cfg.get('KA', 4), cfg.get('KB', 6)
    FPIN = cfg.get('FPIN', True)
    FP0 = cfg.get('FP0', 2)
    FPS = cfg.get('FPS', 1)

    def sc(name):
        return jax.named_scope(name) if scopes else contextlib.nullcontext()

    def kernel(x_hbm, wqkv_hbm, wo_hbm, w1_hbm, w3_hbm, w2_hbm, c_hbm, wmod_hbm, out_hbm,
               x_v, wqkv_v, wo_v, w1_v, w3_v, w2_v, c_v, wm_v, wmc_v,
               mod_v, modc_v, ct_v, h_i, o_i, halo_v, y_v, x1_v, h2_i, acc_v, out_v, sems, osem, msem, z_s):
        def cp(src, dst, k):
            return pltpu.make_async_copy(src, dst, sems.at[k])

        def tile_cps(src, dst, j0, j1, k):
            return [cp(src.at[:, j * 128:(j + 1) * 128], dst.at[j], k) for j in range(j0, j1)]

        def start(cs):
            for c_ in cs:
                c_.start()

        def wait(cs, name=None):
            with (sc(name) if name else contextlib.nullcontext()):
                for c_ in cs:
                    c_.wait()

        def wm_cp(p):
            return cp(wmod_hbm.at[:, pl.ds(pl.multiple_of(p * D, D), D)], wm_v.at[p], 12 + p)

        def wmc_cp(c):
            col = pl.multiple_of(2 * D + c * 512, 512)
            return pltpu.make_async_copy(wmod_hbm.at[:, pl.ds(col, 512)], wmc_v.at[c], msem.at[c])

        c_cp = cp(c_hbm, c_v, 0)
        x0_cp = cp(x_hbm.at[0:TM], x_v.at[0:TM], 1)
        x1_cp = cp(x_hbm.at[TM:2 * TM], x_v.at[TM:2 * TM], 2)
        x2_cp = cp(x_hbm.at[2 * TM:3 * TM], x_v.at[2 * TM:3 * TM], 10)
        x3_cp = cp(x_hbm.at[3 * TM:S], x_v.at[3 * TM:S], 11)
        wq_cps = tile_cps(wqkv_hbm, wqkv_v, 0, 8, 3)
        def half_cps(j0, hh, k):
            rows = pl.ds(hh * 512, 512)
            return [cp(wqkv_hbm.at[rows, j * 128:(j + 1) * 128], wqkv_v.at[j, rows], k) for j in range(j0, j0 + 8)]
        wk_cps = [half_cps(8, 0, 4), half_cps(8, 1, 15)]
        wv_cps = [half_cps(16, 0, 5), half_cps(16, 1, 16)]
        wo_cps = tile_cps(wo_hbm, wo_v, 0, 8, 6)
        if TILED:
            w1_cps = tile_cps(w1_hbm, w1_v, 0, F // 128, 7)
            w3_cps = tile_cps(w3_hbm, w3_v, 0, F // 128, 8)
            w2_cps = tile_cps(w2_hbm, w2_v, 0, DT, 9)
            w1_i, w3_i, w2_i = w1_v.bitcast(i32), w3_v.bitcast(i32), w2_v.bitcast(i32)
        else:
            w1_cps, w3_cps, w2_cps = [cp(w1_hbm, w1_v, 7)], [cp(w3_hbm, w3_v, 8)], [cp(w2_hbm, w2_v, 9)]

        start([c_cp, x0_cp] + wq_cps + [wm_cp(1), wm_cp(0)] + wk_cps[0] + wk_cps[1])

        wqkv_i = wqkv_v.bitcast(i32)
        wo_i = wo_v.bitcast(i32)

        halo_v[...] = jnp.zeros((16, HALO, 128), f32)
        acc_v[...] = jnp.zeros_like(acc_v)
        z_s[0] = jnp.int32(0)

        c_cp.wait()
        cf = c_v[...].astype(f32)
        sf = (cf * jax.nn.sigmoid(cf)).astype(bf16)
        sc16 = jnp.broadcast_to(sf, (16, D))
        sf = sf.astype(f32)
        for t in range(DT):
            ct_v[t * 128:(t + 1) * 128, :] = jnp.broadcast_to(sf[:, t * 128:(t + 1) * 128], (128, 128)).T

        def zvec():
            return jnp.full((8, 128), z_s[0], i32)

        def ldw(wi, j, pin=None):
            w = wi[j]
            if pin is not None:
                w = jnp.concatenate([w[0:8] | (pltpu.bitcast(pin, i32) & zvec()), w[8:]], axis=0)
            return pltpu.bitcast(w, bf16)

        def mm(lhs, wi, j, pin=None):
            return jnp.dot(lhs, ldw(wi, j, pin), preferred_element_type=f32)

        def mod_fin(p, pins=None):
            if pins is None:
                r = jnp.dot(sc16, wm_v[p], preferred_element_type=f32)[0:8]
            else:
                wmi = wm_v.bitcast(i32)
                rs = []
                for n in range(DT):
                    w = wmi[p, :, n * 128:(n + 1) * 128]
                    w = jnp.concatenate([w[0:8] | (pins[n] & zvec()), w[8:]], axis=0)
                    rs.append(jnp.dot(sc16, pltpu.bitcast(w, bf16), preferred_element_type=f32)[0:8])
                r = jnp.concatenate(rs, axis=1)
            mod_v[p] = r + jnp.where(p == 1, 1.0, 0.0)

        def mod(k):
            if k >= 2:
                return jnp.concatenate([modc_v[(k - 2) * 8 + j, 0:1, :] for j in range(DT)], axis=1)
            return mod_v[k, 0:1, :]

        def ln1_val(t):
            r = pl.ds(pl.multiple_of(t * TM, TM), TM)
            return _pack((_normalize(x_v[r, :].astype(f32)) * mod(1) + mod(0)).astype(bf16))

        def ln_pins(hw):
            rp = hw[0].shape[0] // 8
            return [_or_all([t[n * rp:(n + 1) * rp] for t in hw]) for n in range(8)]

        def st_tiles(dst, tiles, rows=slice(None)):
            for j, t in enumerate(tiles):
                dst[j, rows, :] = t

        def o_phase(t, pins):
            r = pl.ds(pl.multiple_of(t * TM, TM), TM)
            o = _ld(o_i)
            for n in range(DT):
                cs = slice(n * 128, (n + 1) * 128)
                y = mm(o, wo_i, n, pins[n])
                y_v[r, cs] = y

        def kv_tile(h, sec, n, pin=None):
            y = mm(h, wqkv_i, 8 * sec + n, pin)
            full = jnp.concatenate([halo_v[8 * (sec - 1) + n], y], axis=0)
            halo_v[8 * (sec - 1) + n] = y[TM - HALO:]
            return full

        def mod_chunk(c):
            w = wmc_v[c].astype(f32)
            outs = []
            for e in range(4):
                p = w[:, e * 128:(e + 1) * 128] * ct_v[...]
                acc = None
                for r in range(0, D, 8):
                    acc = p[r:r + 8] if acc is None else acc + p[r:r + 8]
                for s in (4, 2, 1):
                    acc = acc + pltpu.roll(acc, s, 0)
                outs.append(acc)
            for e in range(4):
                tau = c * 4 + e
                modc_v[tau] = outs[e] + jnp.where(tau // 8 == 2, 1.0, 0.0)
            return outs

        with sc('wq_perm'):
            wait(wq_cps)
            _permute_cols(wqkv_i, 0, PG)
        with sc('xhat0'):
            x0_cp.wait()
            x1_v[0] = _normalize(x_v[0:TM, :].astype(f32))
        with sc('mod_a'):
            def mbody(t, carry):
                wm_cp(1 - t).wait()

                @pl.when(t == 0)
                def _():
                    start([x1_cp] + wv_cps[0])
                mod_fin(1 - t)
                return carry
            lax.fori_loop(0, 2, mbody, 0)

        with sc('A0'):
            _st(h_i, (x1_v[0] * mod(1) + mod(0)).astype(bf16))
            h = _ld(h_i)
            q = []
            for n in range(8):
                if n == QA:
                    wait(wk_cps[0], 'w_wk0')
                    start(wv_cps[1])
                    _permute_cols(wqkv_i, 8, PG, 0, 256)
                if n == QB:
                    wait(wk_cps[1], 'w_wk1')
                    start(wo_cps)
                    _permute_cols(wqkv_i, 8, PG, 256, 512)
                q.append(mm(h, wqkv_i, n))
            wait([x1_cp], 'w_x1')
            hn = ln1_val(1)
            pins = ln_pins(hn)
            if KA == 4:
                pins = [None, pins[0] | pins[1], pins[2] | pins[3] | pins[4], pins[5] | pins[6] | pins[7]] + [None] * 4
            else:
                pins = [None] + [_or_all([p_ for p_ in pins[(n - 1) * 8 // (KA - 1):n * 8 // (KA - 1)]]) for n in range(1, KA)] + [None] * (8 - KA)
            kfull = []
            for n in range(8):
                if n == KA:
                    wait(wv_cps[0], 'w_wv0')
                    _permute_cols(wqkv_i, 16, PG, 0, 256)
                if n == KB:
                    wait(wv_cps[1], 'w_wv1')
                    start([x2_cp, wmc_cp(0), x3_cp])
                    _permute_cols(wqkv_i, 16, PG, 256, 512)
                kfull.append(kv_tile(h, 1, n, pins[n]))
            ps, inv = _softmax_weights(q, kfull, 0)
            vfull = []
            VS = cfg.get('VS', 4)
            for n in range(8):
                pin = None
                if n == VS:
                    wait(wo_cps, 'w_wo')
                    rpins = _permute_rows(wo_i)
                if 1 <= n < VS:
                    lo, hi = (n - 1) * TM // (VS - 1) // 8 * 8, n * TM // (VS - 1) // 8 * 8
                    pin = _or_all([inv[lo:hi]])
                elif n > VS:
                    k_ = 8 - VS - 1
                    pin = _or_all(rpins[(n - VS - 1) * 8 // k_:(n - VS) * 8 // k_])
                vfull.append(kv_tile(h, 2, n, pin))
            of = [_pv(ps, vfull[j]) for j in range(DT)]
            _st(o_i, jnp.concatenate([o_.astype(bf16) for o_ in of], axis=1))
            st_tiles(h_i, hn)

        def a_body(i):
            h = _ld(h_i)
            mouts = mod_chunk(i - 1)
            q = [mm(h, wqkv_i, n, mouts[n - 2] if 2 <= n < 6 else None) for n in range(8)]
            hn = ln1_val(jnp.minimum(i + 1, NT - 1))
            pins = ln_pins(hn)
            kfull = [kv_tile(h, 1, n, pins[n]) for n in range(8)]
            ps, inv = _softmax_weights(q, kfull, i * TM)
            vfull = [kv_tile(h, 2, n) for n in range(8)]
            of = [_pv(ps, vfull[j]) for j in range(DT)]
            o_phase(i - 1, [_or_all([of[n]]) for n in range(DT)])
            _st(o_i, jnp.concatenate([o_.astype(bf16) for o_ in of], axis=1))
            st_tiles(h_i, hn)

        def a_loop(i, carry):
            wmc_cp(i - 1).wait()
            for it_, waits, starts in ((1, [x2_cp], [wmc_cp(c) for c in range(1, 8)]),
                                       (2, [x3_cp], w1_cps), (4, [], w3_cps), (6, [], w2_cps)):
                @pl.when(i == it_)
                def _(waits=waits, starts=starts):
                    wait(waits)
                    start(starts)

            with sc('Ait'):
                a_body(i)
            return carry
        lax.fori_loop(1, NT, a_loop, 0)

        with sc('wo7'):
            wait(w1_cps + w3_cps + w2_cps)
            wmc_cp(7).wait()
            x10 = x_v[0:TM, :].astype(f32) + mod(2) * y_v[0:TM, :]
            if not cfg.get('RECOMP', True):
                x1_v[0] = x10
            h20 = _pack((_normalize(x10) * mod(4) + mod(3)).astype(bf16))
            mouts = mod_chunk(7)
            lp = ln_pins(h20)
            mp = [pltpu.bitcast(m_, i32) for m_ in mouts]
            w7 = cfg.get('W7', 1)
            if w7 == 0:
                pins = [None, mp[0] | mp[1], mp[2] | mp[3], lp[0] | lp[1], lp[2] | lp[3], lp[4] | lp[5], lp[6] | lp[7], None]
            elif w7 == 1:
                pins = [None, lp[0] | lp[1], lp[2] | lp[3], lp[4] | lp[5], lp[6] | lp[7], mp[0] | mp[1], mp[2] | mp[3], None]
            elif w7 == 2:
                pins = [None, None, lp[0] | lp[1] | lp[2], lp[3] | lp[4] | lp[5], lp[6] | lp[7], mp[0] | mp[1], mp[2] | mp[3], None]
            else:
                pins = [None, mp[0], mp[1] | lp[0], mp[2] | lp[1] | lp[2], mp[3] | lp[3] | lp[4], lp[5] | lp[6], lp[7], None]
            o_phase(NT - 1, pins)
            st_tiles(h2_i.at[0], h20)

        def f_iter(it):
            i = it // 2
            half = it % 2
            r = pl.ds(pl.multiple_of(i * TM, TM), TM)
            h2 = _ld(h2_i.at[i % 2])
            hm = TM // 2
            t = jnp.minimum(i + 1, NT - 1)
            rr = pl.ds(pl.multiple_of(t * TM + half * hm, hm), hm)
            xn = x_v[rr, :].astype(f32) + mod(2) * y_v[rr, :]
            hn = _pack((_normalize(xn) * mod(4) + mod(3)).astype(bf16))
            pins = ln_pins(hn)
            acc = acc_v[...] * half.astype(f32)
            c0 = pl.multiple_of(half * FH, FH)
            for c in range(FH // FC):
                if TILED:
                    t0 = half * (FH // 128) + c * (FC // 128)
                    nt_ = FC // 128

                    def lt(wi, pp):
                        tiles = []
                        for e in range(nt_):
                            w = wi[t0 + e]
                            if pp is not None and pp.get(e) is not None:
                                w = jnp.concatenate([w[0:8] | (pp[e] & zvec()), w[8:]], axis=0)
                            tiles.append(pltpu.bitcast(w, bf16))
                        return jnp.concatenate(tiles, axis=1)
                    pp = {FP0 + n * FPS: pins[n] for n in range(8)} if (FPIN and c == 0) else None
                    g = jnp.dot(h2, lt(w1_i, pp), preferred_element_type=f32)
                    u = jnp.dot(h2, lt(w3_i, None), preferred_element_type=f32)
                    a = (_silu(g) * u).astype(bf16)
                    kr = pl.ds(pl.multiple_of(t0 * 64, 64), FC // 2)
                    w2 = jnp.concatenate([pltpu.bitcast(w2_i[j, kr, :], bf16) for j in range(DT)], axis=1)
                    acc = acc + jnp.dot(a, w2, preferred_element_type=f32)
                    continue
                cs = pl.ds(c0 + c * FC, FC)
                g = jnp.dot(h2, w1_v[:, cs], preferred_element_type=f32)
                u = jnp.dot(h2, w3_v[:, cs], preferred_element_type=f32)
                a = (_silu(g) * u).astype(bf16)
                acc = acc + jnp.dot(a, w2_v[cs, :], preferred_element_type=f32)
            acc_v[...] = acc
            if cfg.get('RECOMP', True):
                x1 = x_v[r, :].astype(f32) + mod(2) * y_v[r, :]
                out_v[r, :] = (x1 + mod(5) * acc).astype(out_v.dtype)
            else:
                out_v[r, :] = (x1_v[i % 2] + mod(5) * acc).astype(out_v.dtype)
                x1_v[(i + 1) % 2, pl.ds(pl.multiple_of(half * hm, hm), hm), :] = xn
            st_tiles(h2_i.at[(i + 1) % 2], hn, rows=pl.ds(pl.multiple_of(half * (hm // 2), hm // 2), hm // 2))

            @pl.when(half == 1)
            def _():
                pltpu.make_async_copy(out_v.at[r], out_hbm.at[r], osem.at[i]).start()

        def f_loop(it, carry):
            with sc('Fit'):
                f_iter(it)
            return carry
        lax.fori_loop(0, 2 * NT, f_loop, 0)
        with sc('tail'):
            for i in range(NT):
                r = pl.ds(i * TM, TM)
                pltpu.make_async_copy(out_v.at[r], out_hbm.at[r], osem.at[i]).wait()

    return kernel


def build(debug=False, **cfg):
    kern = make_kernel(cfg)
    odt = f32 if debug else bf16

    def f(A_x, A_wqkv, A_wo, B_w1, B_w3, B_w2, c, w_mod):
        x = A_x.reshape(S, D)
        anyspec = pl.BlockSpec(memory_space=pl.ANY)
        out = pl.pallas_call(
            kern,
            in_specs=[anyspec] * 8,
            out_specs=anyspec,
            out_shape=jax.ShapeDtypeStruct((S, D), odt),
            scratch_shapes=[
                pltpu.VMEM((S, D), bf16),
                pltpu.VMEM((3 * DT, D, 128), bf16),
                pltpu.VMEM((DT, D, 128), bf16),
                *([pltpu.VMEM((F // 128, D, 128), bf16), pltpu.VMEM((F // 128, D, 128), bf16), pltpu.VMEM((DT, F, 128), bf16)] if cfg.get('TILED', True)
                  else [pltpu.VMEM((D, F), bf16), pltpu.VMEM((D, F), bf16), pltpu.VMEM((F, D), bf16)]),
                pltpu.VMEM((1, D), bf16),
                pltpu.VMEM((2, D, D), bf16),
                pltpu.VMEM((8, D, 512), bf16),
                pltpu.VMEM((2, 8, D), f32),
                pltpu.VMEM((32, 8, 128), f32),
                pltpu.VMEM((D, 128), f32),
                pltpu.VMEM((DT, TM // 2, 128), i32),
                pltpu.VMEM((DT, TM // 2, 128), i32),
                pltpu.VMEM((16, HALO, 128), f32),
                pltpu.VMEM((S, D), f32),
                pltpu.VMEM((2, TM, D), f32),
                pltpu.VMEM((2, DT, TM // 2, 128), i32),
                pltpu.VMEM((TM, D), f32),
                pltpu.VMEM((S, D), odt),
                pltpu.SemaphoreType.DMA((17,)),
                pltpu.SemaphoreType.DMA((NT,)),
                pltpu.SemaphoreType.DMA((8,)),
                pltpu.SMEM((1,), i32),
            ],
            compiler_params=pltpu.CompilerParams(vmem_limit_bytes=120 * 2**20),
        )(x, A_wqkv, A_wo, B_w1, B_w3, B_w2, c, w_mod)
        return out.reshape(1, S, D)
    return f


@jax.jit
def pallas_adaLN_cond__sliding_local_dilated__glu_gated_swiglu__prompt_kernel(
    A_x: jax.Array,
    A_wqkv: jax.Array,
    A_wo: jax.Array,
    B_x: jax.Array,
    B_w1: jax.Array,
    B_w3: jax.Array,
    B_w2: jax.Array,
    c: jax.Array,
    w_mod: jax.Array,
):
    del B_x
    return build()(A_x, A_wqkv, A_wo, B_w1, B_w3, B_w2, c, w_mod)
```

```python
import contextlib
import jax
import jax.numpy as jnp
from jax import lax
from jax.experimental import pallas as pl
from jax.experimental.pallas import tpu as pltpu

S, D, H, DH, F = 2048, 1024, 32, 32, 3584
W, DIL = 8, 2
HALO = 16
DT = D // 128
TM = 256
NT = S // TM
f32, bf16, i32 = jnp.float32, jnp.bfloat16, jnp.int32


def _normalize(xf):
    mean = jnp.sum(xf, axis=-1, keepdims=True) * (1.0 / D)
    xc = xf - mean
    var = jnp.sum(xc * xc, axis=-1, keepdims=True) * (1.0 / D)
    return xc * lax.rsqrt(var + 1e-5)


def _silu(g):
    hg = 0.5 * g
    return hg * jnp.tanh(hg) + hg


def _ld(wi):
    return jnp.concatenate([pltpu.bitcast(wi[j], bf16) for j in range(wi.shape[0])], axis=1)


def _st(dst, val, rows=slice(None)):
    for j in range(val.shape[1] // 128):
        dst[j, rows, :] = pltpu.bitcast(val[:, j * 128:(j + 1) * 128], i32)


def _pack(val):
    return [pltpu.bitcast(val[:, j * 128:(j + 1) * 128], i32) for j in range(val.shape[1] // 128)]


def _or_all(vals):
    t = None
    for v in vals:
        v = pltpu.bitcast(v, i32)
        for r in range(0, v.shape[0], 8):
            t = v[r:r + 8] if t is None else t | v[r:r + 8]
    return t


def _xor_net(vs, masks):
    vs = list(vs)
    for b in range(3):
        nv = list(vs)
        for u in range(8):
            if not (u >> b) & 1:
                p = u | (1 << b)
                nv[u] = jnp.where(masks[b], vs[p], vs[u])
                nv[p] = jnp.where(masks[b], vs[u], vs[p])
        vs = nv
    return vs


def _permute_cols(wi, t0, G, g0=0, g1=512):
    R = 8 * G
    lane = lax.broadcasted_iota(i32, (R, 128), 1)
    masks = [((lane >> (2 + b)) & 1) == 1 for b in range(3)]
    r, j, a = lane >> 5, (lane >> 2) & 7, lane & 3
    idx = [a * 32 + (j ^ u) * 4 + r for u in range(8)]
    for g in range(g0, g1, R):
        rows = pl.ds(g, R)
        src = [wi[t0 + t, rows, :] for t in range(8)]
        mer = _xor_net(src, masks)
        per = [jnp.take_along_axis(mer[u], idx[u], axis=1) for u in range(8)]
        dst = _xor_net(per, masks)
        for t in range(8):
            wi[t0 + t, rows, :] = dst[t]


def _permute_rows(wi):
    sub = lax.broadcasted_iota(i32, (8, 128), 0)
    low = [((sub >> b) & 1) == 0 for b in range(3)]
    done = []
    for j in range(DT):
        tgt = [None] * 64
        for eh in range(2):
            for mh in range(2):
                for par in range(2):
                    vs = []
                    for m in range(8 * mh, 8 * mh + 8):
                        A = wi[j, pl.ds((2 * m) * 16 + 8 * eh, 8), :]
                        B = wi[j, pl.ds((2 * m + 1) * 16 + 8 * eh, 8), :]
                        vs.append((A & 0xFFFF) | (B << 16) if par == 0
                                  else lax.shift_right_logical(A, 16) | (B & jnp.int32(-65536)))
                    for b in range(3):
                        s = 1 << b
                        nv = list(vs)
                        for u in range(8):
                            if not (u >> b) & 1:
                                p = u | s
                                nv[u] = jnp.where(low[b], vs[u], pltpu.roll(vs[p], s, 0))
                                nv[p] = jnp.where(low[b], pltpu.roll(vs[u], 8 - s, 0), vs[p])
                        vs = nv
                    for e in range(8):
                        tgt[(2 * (8 * eh + e) + par) * 2 + mh] = vs[e]
        wi[j] = jnp.concatenate(tgt, axis=0)
        done.append(tgt[63])
    return done


def _windows(full, M):
    outs = [None] * W
    for s in range(4):
        r = full if s == 0 else pltpu.roll(full, DIL * s, 0)
        outs[s] = r[HALO:HALO + M]
        outs[s + 4] = r[HALO - 8:HALO - 8 + M]
    return outs


def _softmax_weights(q, kfull, pos0):
    scale = DH ** -0.5
    pos = pos0 + lax.broadcasted_iota(i32, (TM, 128), 0)
    acc = [None] * W
    for j in range(DT):
        ks = _windows(kfull[j], TM)
        for w in range(W):
            p = q[j] * ks[w]
            acc[w] = p if acc[w] is None else acc[w] + p
    logits = []
    for w in range(W):
        a = acc[w]
        a = a + pltpu.roll(a, 64, 1)
        a = a + pltpu.roll(a, 32, 1)
        a = a * scale
        if w > 0:
            a = jnp.where(pos >= DIL * w, a, -1e9)
        logits.append(a)
    m = logits[0]
    for w in range(1, W):
        m = jnp.maximum(m, logits[w])
    es = [jnp.exp(l - m) for l in logits]
    den = es[0]
    for w in range(1, W):
        den = den + es[w]
    inv = 1.0 / den
    return [e * inv for e in es], inv


def _pv(ps, vfull, R=32):
    outs = []
    for r0 in range(0, TM, R):
        vs = _windows(vfull[r0:r0 + HALO + R], R)
        acc = None
        for w in range(W):
            p = ps[w][r0:r0 + R] * vs[w]
            acc = p if acc is None else acc + p
        outs.append(acc)
    return jnp.concatenate(outs, axis=0)


def make_kernel(cfg):
    FH = F // 2
    FC = cfg.get('FC', 1792)
    PG = cfg.get('PG', 8)
    scopes = cfg.get('scopes', False)
    TILED = cfg.get('TILED', True)
    QA, QB, KA, KB = cfg.get('QA', 3), cfg.get('QB', 6), cfg.get('KA', 4), cfg.get('KB', 6)
    FPIN = cfg.get('FPIN', True)
    FP0 = cfg.get('FP0', 2)
    FPS = cfg.get('FPS', 1)

    def sc(name):
        return jax.named_scope(name) if scopes else contextlib.nullcontext()

    def kernel(x_hbm, wqkv_hbm, wo_hbm, w1_hbm, w3_hbm, w2_hbm, c_hbm, wmod_hbm, out_hbm,
               x_v, wqkv_v, wo_v, w1_v, w3_v, w2_v, c_v, wm_v, wmc_v,
               mod_v, modc_v, ct_v, h_i, o_i, halo_v, y_v, x1_v, h2_i, acc_v, out_v, sems, osem, msem, z_s):
        def cp(src, dst, k):
            return pltpu.make_async_copy(src, dst, sems.at[k])

        def tile_cps(src, dst, j0, j1, k):
            return [cp(src.at[:, j * 128:(j + 1) * 128], dst.at[j], k) for j in range(j0, j1)]

        def start(cs):
            for c_ in cs:
                c_.start()

        def wait(cs, name=None):
            with (sc(name) if name else contextlib.nullcontext()):
                for c_ in cs:
                    c_.wait()

        def wm_cp(p):
            return cp(wmod_hbm.at[:, pl.ds(pl.multiple_of(p * 512, 512), 512)], wm_v.at[p], 17 + p)

        def wmc_cp(c):
            col = pl.multiple_of(2 * D + c * 512, 512)
            return pltpu.make_async_copy(wmod_hbm.at[:, pl.ds(col, 512)], wmc_v.at[c], msem.at[c])

        c_cp = cp(c_hbm, c_v, 0)
        x0_cp = cp(x_hbm.at[0:TM], x_v.at[0:TM], 1)
        x1_cp = cp(x_hbm.at[TM:2 * TM], x_v.at[TM:2 * TM], 2)
        x2_cp = cp(x_hbm.at[2 * TM:3 * TM], x_v.at[2 * TM:3 * TM], 10)
        x3_cp = cp(x_hbm.at[3 * TM:S], x_v.at[3 * TM:S], 11)
        wq_cps = tile_cps(wqkv_hbm, wqkv_v, 0, 8, 3)
        def half_cps(j0, hh, k):
            rows = pl.ds(hh * 512, 512)
            return [cp(wqkv_hbm.at[rows, j * 128:(j + 1) * 128], wqkv_v.at[j, rows], k) for j in range(j0, j0 + 8)]
        wk_cps = [half_cps(8, 0, 4), half_cps(8, 1, 15)]
        wv_cps = [half_cps(16, 0, 5), half_cps(16, 1, 16)]
        wo_cps = tile_cps(wo_hbm, wo_v, 0, 8, 6)
        if TILED:
            w1_cps = tile_cps(w1_hbm, w1_v, 0, F // 128, 7)
            w3_cps = tile_cps(w3_hbm, w3_v, 0, F // 128, 8)
            w2_cps = tile_cps(w2_hbm, w2_v, 0, DT, 9)
            w1_i, w3_i, w2_i = w1_v.bitcast(i32), w3_v.bitcast(i32), w2_v.bitcast(i32)
        else:
            w1_cps, w3_cps, w2_cps = [cp(w1_hbm, w1_v, 7)], [cp(w3_hbm, w3_v, 8)], [cp(w2_hbm, w2_v, 9)]

        start([c_cp, x0_cp] + wq_cps + [wm_cp(p_) for p_ in range(4)] + wk_cps[0] + wk_cps[1])

        wqkv_i = wqkv_v.bitcast(i32)
        wo_i = wo_v.bitcast(i32)

        halo_v[...] = jnp.zeros((16, HALO, 128), f32)
        acc_v[...] = jnp.zeros_like(acc_v)
        z_s[0] = jnp.int32(0)

        c_cp.wait()
        cf = c_v[...].astype(f32)
        sf = (cf * jax.nn.sigmoid(cf)).astype(bf16)
        sc16 = jnp.broadcast_to(sf, (16, D))
        sf = sf.astype(f32)
        for t in range(DT):
            ct_v[t * 128:(t + 1) * 128, :] = jnp.broadcast_to(sf[:, t * 128:(t + 1) * 128], (128, 128)).T

        def zvec():
            return jnp.full((8, 128), z_s[0], i32)

        def ldw(wi, j, pin=None):
            w = wi[j]
            if pin is not None:
                w = jnp.concatenate([w[0:8] | (pltpu.bitcast(pin, i32) & zvec()), w[8:]], axis=0)
            return pltpu.bitcast(w, bf16)

        def mm(lhs, wi, j, pin=None):
            return jnp.dot(lhs, ldw(wi, j, pin), preferred_element_type=f32)

        def mod_fin(p):
            r = jnp.dot(sc16, wm_v[p], preferred_element_type=f32)[0:8]
            mod_v[p] = r + jnp.where(p >= 2, 1.0, 0.0)

        def mod(k):
            if k >= 2:
                return jnp.concatenate([modc_v[(k - 2) * 8 + j, 0:1, :] for j in range(DT)], axis=1)
            return jnp.concatenate([mod_v[2 * k, 0:1, :], mod_v[2 * k + 1, 0:1, :]], axis=1)

        def ln1_val(t):
            r = pl.ds(pl.multiple_of(t * TM, TM), TM)
            return _pack((_normalize(x_v[r, :].astype(f32)) * mod(1) + mod(0)).astype(bf16))

        def ln_pins(hw):
            rp = hw[0].shape[0] // 8
            return [_or_all([t[n * rp:(n + 1) * rp] for t in hw]) for n in range(8)]

        def st_tiles(dst, tiles, rows=slice(None)):
            for j, t in enumerate(tiles):
                dst[j, rows, :] = t

        def o_phase(t, pins):
            r = pl.ds(pl.multiple_of(t * TM, TM), TM)
            o = _ld(o_i)
            for n in range(DT):
                cs = slice(n * 128, (n + 1) * 128)
                y = mm(o, wo_i, n, pins[n])
                y_v[r, cs] = y

        def kv_tile(h, sec, n, pin=None):
            y = mm(h, wqkv_i, 8 * sec + n, pin)
            full = jnp.concatenate([halo_v[8 * (sec - 1) + n], y], axis=0)
            halo_v[8 * (sec - 1) + n] = y[TM - HALO:]
            return full

        def mod_chunk(c):
            w = wmc_v[c].astype(f32)
            outs = []
            for e in range(4):
                p = w[:, e * 128:(e + 1) * 128] * ct_v[...]
                acc = None
                for r in range(0, D, 8):
                    acc = p[r:r + 8] if acc is None else acc + p[r:r + 8]
                for s in (4, 2, 1):
                    acc = acc + pltpu.roll(acc, s, 0)
                outs.append(acc)
            for e in range(4):
                tau = c * 4 + e
                modc_v[tau] = outs[e] + jnp.where(tau // 8 == 2, 1.0, 0.0)
            return outs

        with sc('wq_perm'):
            wait(wq_cps)
            _permute_cols(wqkv_i, 0, PG)
        with sc('xhat0'):
            x0_cp.wait()
            x1_v[0] = _normalize(x_v[0:TM, :].astype(f32))
        with sc('mod_a'):
            def mbody(t, carry):
                wm_cp(t).wait()

                @pl.when(t == 1)
                def _():
                    start([x1_cp] + wv_cps[0])
                mod_fin(t)
                return carry
            lax.fori_loop(0, 4, mbody, 0)

        with sc('A0'):
            _st(h_i, (x1_v[0] * mod(1) + mod(0)).astype(bf16))
            h = _ld(h_i)
            q = []
            for n in range(8):
                if n == QA:
                    wait(wk_cps[0], 'w_wk0')
                    start(wv_cps[1])
                    _permute_cols(wqkv_i, 8, PG, 0, 256)
                if n == QB:
                    wait(wk_cps[1], 'w_wk1')
                    start(wo_cps)
                    _permute_cols(wqkv_i, 8, PG, 256, 512)
                q.append(mm(h, wqkv_i, n))
            wait([x1_cp], 'w_x1')
            hn = ln1_val(1)
            pins = ln_pins(hn)
            if KA == 4:
                pins = [None, pins[0] | pins[1], pins[2] | pins[3] | pins[4], pins[5] | pins[6] | pins[7]] + [None] * 4
            else:
                pins = [None] + [_or_all([p_ for p_ in pins[(n - 1) * 8 // (KA - 1):n * 8 // (KA - 1)]]) for n in range(1, KA)] + [None] * (8 - KA)
            kfull = []
            for n in range(8):
                if n == KA:
                    wait(wv_cps[0], 'w_wv0')
                    _permute_cols(wqkv_i, 16, PG, 0, 256)
                if n == KB:
                    wait(wv_cps[1], 'w_wv1')
                    start([x2_cp, wmc_cp(0), x3_cp])
                    _permute_cols(wqkv_i, 16, PG, 256, 512)
                kfull.append(kv_tile(h, 1, n, pins[n]))
            ps, inv = _softmax_weights(q, kfull, 0)
            vfull = []
            VS = cfg.get('VS', 4)
            RP0 = cfg.get('RP0', 5)
            for n in range(8):
                pin = None
                if n == VS:
                    wait(wo_cps, 'w_wo')
                    rpins = _permute_rows(wo_i)
                if 1 <= n < VS:
                    lo, hi = (n - 1) * TM // (VS - 1) // 8 * 8, n * TM // (VS - 1) // 8 * 8
                    pin = _or_all([inv[lo:hi]])
                elif n >= RP0:
                    k_ = 8 - RP0
                    pin = _or_all(rpins[(n - RP0) * 8 // k_:(n - RP0 + 1) * 8 // k_])
                vfull.append(kv_tile(h, 2, n, pin))
            of = [_pv(ps, vfull[j]) for j in range(DT)]
            _st(o_i, jnp.concatenate([o_.astype(bf16) for o_ in of], axis=1))
            st_tiles(h_i, hn)

        def a_body(i):
            h = _ld(h_i)
            mouts = mod_chunk(i - 1)
            mp = [pltpu.bitcast(m_, i32) for m_ in mouts]
            hn = ln1_val(jnp.minimum(i + 1, NT - 1))
            lp = ln_pins(hn)
            mode = cfg.get('AM', 3)
            qp, kp, op = [None] * 8, [None] * 8, [None] * 8
            if mode == 0:
                qp = [mp[n - 2] if 2 <= n < 6 else None for n in range(8)]
                kp = lp
            elif mode == 1:
                qp = [mp[n - 2] if 2 <= n < 6 else None for n in range(8)]
                op = lp
            elif mode == 2:
                qp = [None, mp[0] | mp[1], mp[2] | mp[3], lp[0] | lp[1], lp[2] | lp[3], lp[4] | lp[5], lp[6] | lp[7], None]
            elif mode == 3:
                qp = [None] + [lp[n] for n in range(6)] + [lp[6] | lp[7]]
                op = [None, None, mp[0], mp[1], mp[2], mp[3], None, None]
            elif mode == 4:
                qp = [None, mp[0], mp[1], mp[2], mp[3], lp[0], lp[1], lp[2]]
                kp = [lp[3], lp[4] | lp[5], lp[6] | lp[7]] + [None] * 5
            elif mode == 5:
                qp = [None, lp[0] | lp[1], lp[2] | lp[3], lp[4] | lp[5], lp[6] | lp[7], mp[0] | mp[1], mp[2] | mp[3], None]
            q = [mm(h, wqkv_i, n, qp[n]) for n in range(8)]
            kfull = [kv_tile(h, 1, n, kp[n]) for n in range(8)]
            ps, inv = _softmax_weights(q, kfull, i * TM)
            vfull = [kv_tile(h, 2, n) for n in range(8)]
            of = [_pv(ps, vfull[j]) for j in range(DT)]
            opins = [_or_all([of[n]]) if op[n] is None else (_or_all([of[n]]) | op[n]) for n in range(DT)]
            o_phase(i - 1, opins)
            _st(o_i, jnp.concatenate([o_.astype(bf16) for o_ in of], axis=1))
            st_tiles(h_i, hn)

        def a_loop(i, carry):
            wmc_cp(i - 1).wait()
            for it_, waits, starts in ((1, [x2_cp], [wmc_cp(c) for c in range(1, 8)]),
                                       (2, [x3_cp], w1_cps), (4, [], w3_cps), (6, [], w2_cps)):
                @pl.when(i == it_)
                def _(waits=waits, starts=starts):
                    wait(waits)
                    start(starts)

            with sc('Ait'):
                a_body(i)
            return carry
        lax.fori_loop(1, NT, a_loop, 0)

        with sc('wo7'):
            wait(w1_cps + w3_cps + w2_cps)
            wmc_cp(7).wait()
            x10 = x_v[0:TM, :].astype(f32) + mod(2) * y_v[0:TM, :]
            if not cfg.get('RECOMP', True):
                x1_v[0] = x10
            h20 = _pack((_normalize(x10) * mod(4) + mod(3)).astype(bf16))
            mouts = mod_chunk(7)
            lp = ln_pins(h20)
            mp = [pltpu.bitcast(m_, i32) for m_ in mouts]
            w7 = cfg.get('W7', 1)
            if w7 == 0:
                pins = [None, mp[0] | mp[1], mp[2] | mp[3], lp[0] | lp[1], lp[2] | lp[3], lp[4] | lp[5], lp[6] | lp[7], None]
            elif w7 == 1:
                pins = [None, lp[0] | lp[1], lp[2] | lp[3], lp[4] | lp[5], lp[6] | lp[7], mp[0] | mp[1], mp[2] | mp[3], None]
            elif w7 == 2:
                pins = [None, None, lp[0] | lp[1] | lp[2], lp[3] | lp[4] | lp[5], lp[6] | lp[7], mp[0] | mp[1], mp[2] | mp[3], None]
            else:
                pins = [None, mp[0], mp[1] | lp[0], mp[2] | lp[1] | lp[2], mp[3] | lp[3] | lp[4], lp[5] | lp[6], lp[7], None]
            o_phase(NT - 1, pins)
            st_tiles(h2_i.at[0], h20)

        def f_iter(it):
            i = it // 2
            half = it % 2
            r = pl.ds(pl.multiple_of(i * TM, TM), TM)
            h2 = _ld(h2_i.at[i % 2])
            hm = TM // 2
            t = jnp.minimum(i + 1, NT - 1)
            rr = pl.ds(pl.multiple_of(t * TM + half * hm, hm), hm)
            xn = x_v[rr, :].astype(f32) + mod(2) * y_v[rr, :]
            hn = _pack((_normalize(xn) * mod(4) + mod(3)).astype(bf16))
            pins = ln_pins(hn)
            acc = jnp.where(half == 1, acc_v[...], 0.0)
            c0 = pl.multiple_of(half * FH, FH)
            for c in range(FH // FC):
                if TILED:
                    t0 = half * (FH // 128) + c * (FC // 128)
                    nt_ = FC // 128

                    def lt(wi, pp):
                        tiles = []
                        for e in range(nt_):
                            w = wi[t0 + e]
                            if pp is not None and pp.get(e) is not None:
                                w = jnp.concatenate([w[0:8] | (pp[e] & zvec()), w[8:]], axis=0)
                            tiles.append(pltpu.bitcast(w, bf16))
                        return jnp.concatenate(tiles, axis=1)
                    pp = {FP0 + n * FPS: pins[n] for n in range(8)} if (FPIN and c == 0) else None
                    g = jnp.dot(h2, lt(w1_i, pp), preferred_element_type=f32)
                    u = jnp.dot(h2, lt(w3_i, None), preferred_element_type=f32)
                    a = (_silu(g) * u).astype(bf16)
                    kr = pl.ds(pl.multiple_of(t0 * 64, 64), FC // 2)
                    w2 = jnp.concatenate([pltpu.bitcast(w2_i[j, kr, :], bf16) for j in range(DT)], axis=1)
                    acc = acc + jnp.dot(a, w2, preferred_element_type=f32)
                    continue
                cs = pl.ds(c0 + c * FC, FC)
                g = jnp.dot(h2, w1_v[:, cs], preferred_element_type=f32)
                u = jnp.dot(h2, w3_v[:, cs], preferred_element_type=f32)
                a = (_silu(g) * u).astype(bf16)
                acc = acc + jnp.dot(a, w2_v[cs, :], preferred_element_type=f32)
            acc_v[...] = acc
            if cfg.get('RECOMP', True):
                x1 = x_v[r, :].astype(f32) + mod(2) * y_v[r, :]
                out_v[r, :] = (x1 + mod(5) * acc).astype(out_v.dtype)
            else:
                out_v[r, :] = (x1_v[i % 2] + mod(5) * acc).astype(out_v.dtype)
                x1_v[(i + 1) % 2, pl.ds(pl.multiple_of(half * hm, hm), hm), :] = xn
            st_tiles(h2_i.at[(i + 1) % 2], hn, rows=pl.ds(pl.multiple_of(half * (hm // 2), hm // 2), hm // 2))

            @pl.when(half == 1)
            def _():
                pltpu.make_async_copy(out_v.at[r], out_hbm.at[r], osem.at[i]).start()

        def f_loop(it, carry):
            with sc('Fit'):
                f_iter(it)
            return carry
        lax.fori_loop(0, 2 * NT, f_loop, 0)
        with sc('tail'):
            for i in range(NT):
                r = pl.ds(i * TM, TM)
                pltpu.make_async_copy(out_v.at[r], out_hbm.at[r], osem.at[i]).wait()

    return kernel


def build(debug=False, **cfg):
    kern = make_kernel(cfg)
    odt = f32 if debug else bf16

    def f(A_x, A_wqkv, A_wo, B_w1, B_w3, B_w2, c, w_mod):
        x = A_x.reshape(S, D)
        anyspec = pl.BlockSpec(memory_space=pl.ANY)
        out = pl.pallas_call(
            kern,
            in_specs=[anyspec] * 8,
            out_specs=anyspec,
            out_shape=jax.ShapeDtypeStruct((S, D), odt),
            scratch_shapes=[
                pltpu.VMEM((S, D), bf16),
                pltpu.VMEM((3 * DT, D, 128), bf16),
                pltpu.VMEM((DT, D, 128), bf16),
                *([pltpu.VMEM((F // 128, D, 128), bf16), pltpu.VMEM((F // 128, D, 128), bf16), pltpu.VMEM((DT, F, 128), bf16)] if cfg.get('TILED', True)
                  else [pltpu.VMEM((D, F), bf16), pltpu.VMEM((D, F), bf16), pltpu.VMEM((F, D), bf16)]),
                pltpu.VMEM((1, D), bf16),
                pltpu.VMEM((4, D, 512), bf16),
                pltpu.VMEM((8, D, 512), bf16),
                pltpu.VMEM((4, 8, 512), f32),
                pltpu.VMEM((32, 8, 128), f32),
                pltpu.VMEM((D, 128), f32),
                pltpu.VMEM((DT, TM // 2, 128), i32),
                pltpu.VMEM((DT, TM // 2, 128), i32),
                pltpu.VMEM((16, HALO, 128), f32),
                pltpu.VMEM((S, D), f32),
                pltpu.VMEM((2, TM, D), f32),
                pltpu.VMEM((2, DT, TM // 2, 128), i32),
                pltpu.VMEM((TM, D), f32),
                pltpu.VMEM((S, D), odt),
                pltpu.SemaphoreType.DMA((21,)),
                pltpu.SemaphoreType.DMA((NT,)),
                pltpu.SemaphoreType.DMA((8,)),
                pltpu.SMEM((1,), i32),
            ],
            compiler_params=pltpu.CompilerParams(vmem_limit_bytes=120 * 2**20),
        )(x, A_wqkv, A_wo, B_w1, B_w3, B_w2, c, w_mod)
        return out.reshape(1, S, D)
    return f


@jax.jit
def pallas_adaLN_cond__sliding_local_dilated__glu_gated_swiglu__prompt_kernel(
    A_x: jax.Array,
    A_wqkv: jax.Array,
    A_wo: jax.Array,
    B_x: jax.Array,
    B_w1: jax.Array,
    B_w3: jax.Array,
    B_w2: jax.Array,
    c: jax.Array,
    w_mod: jax.Array,
):
    del B_x
    return build()(A_x, A_wqkv, A_wo, B_w1, B_w3, B_w2, c, w_mod)
```

```python
import contextlib
import jax
import jax.numpy as jnp
from jax import lax
from jax.experimental import pallas as pl
from jax.experimental.pallas import tpu as pltpu

S, D, H, DH, F = 2048, 1024, 32, 32, 3584
W, DIL = 8, 2
HALO = 16
DT = D // 128
TM = 256
NT = S // TM
f32, bf16, i32 = jnp.float32, jnp.bfloat16, jnp.int32


def _normalize(xf):
    mean = jnp.sum(xf, axis=-1, keepdims=True) * (1.0 / D)
    xc = xf - mean
    var = jnp.sum(xc * xc, axis=-1, keepdims=True) * (1.0 / D)
    return xc * lax.rsqrt(var + 1e-5)


def _silu(g):
    hg = 0.5 * g
    return hg * jnp.tanh(hg) + hg


def _ld(wi):
    return jnp.concatenate([pltpu.bitcast(wi[j], bf16) for j in range(wi.shape[0])], axis=1)


def _st(dst, val, rows=slice(None)):
    for j in range(val.shape[1] // 128):
        dst[j, rows, :] = pltpu.bitcast(val[:, j * 128:(j + 1) * 128], i32)


def _pack(val):
    return [pltpu.bitcast(val[:, j * 128:(j + 1) * 128], i32) for j in range(val.shape[1] // 128)]


def _or_all(vals):
    t = None
    for v in vals:
        v = pltpu.bitcast(v, i32)
        for r in range(0, v.shape[0], 8):
            t = v[r:r + 8] if t is None else t | v[r:r + 8]
    return t


def _xor_net(vs, masks):
    vs = list(vs)
    for b in range(3):
        nv = list(vs)
        for u in range(8):
            if not (u >> b) & 1:
                p = u | (1 << b)
                nv[u] = jnp.where(masks[b], vs[p], vs[u])
                nv[p] = jnp.where(masks[b], vs[u], vs[p])
        vs = nv
    return vs


def _permute_cols(wi, t0, G, g0=0, g1=512):
    R = 8 * G
    lane = lax.broadcasted_iota(i32, (R, 128), 1)
    masks = [((lane >> (2 + b)) & 1) == 1 for b in range(3)]
    r, j, a = lane >> 5, (lane >> 2) & 7, lane & 3
    idx = [a * 32 + (j ^ u) * 4 + r for u in range(8)]
    for g in range(g0, g1, R):
        rows = pl.ds(g, R)
        src = [wi[t0 + t, rows, :] for t in range(8)]
        mer = _xor_net(src, masks)
        per = [jnp.take_along_axis(mer[u], idx[u], axis=1) for u in range(8)]
        dst = _xor_net(per, masks)
        for t in range(8):
            wi[t0 + t, rows, :] = dst[t]


def _permute_rows(wi):
    sub = lax.broadcasted_iota(i32, (8, 128), 0)
    low = [((sub >> b) & 1) == 0 for b in range(3)]
    done = []
    for j in range(DT):
        tgt = [None] * 64
        for eh in range(2):
            for mh in range(2):
                for par in range(2):
                    vs = []
                    for m in range(8 * mh, 8 * mh + 8):
                        A = wi[j, pl.ds((2 * m) * 16 + 8 * eh, 8), :]
                        B = wi[j, pl.ds((2 * m + 1) * 16 + 8 * eh, 8), :]
                        vs.append((A & 0xFFFF) | (B << 16) if par == 0
                                  else lax.shift_right_logical(A, 16) | (B & jnp.int32(-65536)))
                    for b in range(3):
                        s = 1 << b
                        nv = list(vs)
                        for u in range(8):
                            if not (u >> b) & 1:
                                p = u | s
                                nv[u] = jnp.where(low[b], vs[u], pltpu.roll(vs[p], s, 0))
                                nv[p] = jnp.where(low[b], pltpu.roll(vs[u], 8 - s, 0), vs[p])
                        vs = nv
                    for e in range(8):
                        tgt[(2 * (8 * eh + e) + par) * 2 + mh] = vs[e]
        wi[j] = jnp.concatenate(tgt, axis=0)
        done.append(tgt[63])
    return done


def _windows(full, M):
    outs = [None] * W
    for s in range(4):
        r = full if s == 0 else pltpu.roll(full, DIL * s, 0)
        outs[s] = r[HALO:HALO + M]
        outs[s + 4] = r[HALO - 8:HALO - 8 + M]
    return outs


def _qk_products(q, kfull, js, acc):
    for j in js:
        ks = _windows(kfull[j], TM)
        for w in range(W):
            p = q[j] * ks[w]
            acc[w] = p if acc[w] is None else acc[w] + p
    return acc


def _softmax_weights(q, kfull, pos0, acc=None, js=range(DT)):
    scale = DH ** -0.5
    pos = pos0 + lax.broadcasted_iota(i32, (TM, 128), 0)
    acc = _qk_products(q, kfull, js, [None] * W if acc is None else acc)
    logits = []
    for w in range(W):
        a = acc[w]
        a = a + pltpu.roll(a, 64, 1)
        a = a + pltpu.roll(a, 32, 1)
        a = a * scale
        if w > 0:
            a = jnp.where(pos >= DIL * w, a, -1e9)
        logits.append(a)
    m = logits[0]
    for w in range(1, W):
        m = jnp.maximum(m, logits[w])
    es = [jnp.exp(l - m) for l in logits]
    den = es[0]
    for w in range(1, W):
        den = den + es[w]
    inv = 1.0 / den
    return [e * inv for e in es], inv


def _pv(ps, vfull, R=32):
    outs = []
    for r0 in range(0, TM, R):
        vs = _windows(vfull[r0:r0 + HALO + R], R)
        acc = None
        for w in range(W):
            p = ps[w][r0:r0 + R] * vs[w]
            acc = p if acc is None else acc + p
        outs.append(acc)
    return jnp.concatenate(outs, axis=0)


def make_kernel(scopes=False):
    FH = F // 2
    PG = 8

    def sc(name):
        return jax.named_scope(name) if scopes else contextlib.nullcontext()

    def kernel(x_hbm, wqkv_hbm, wo_hbm, w1_hbm, w3_hbm, w2_hbm, c_hbm, wmod_hbm, out_hbm,
               x_v, wqkv_v, wo_v, w1_v, w3_v, w2_v, c_v, wm_v, wmc_v,
               mod_v, modc_v, ct_v, h_i, o_i, halo_v, y_v, h2_i, acc_v, out_v, sems, osem, msem, z_s):
        def cp(src, dst, k):
            return pltpu.make_async_copy(src, dst, sems.at[k])

        def tile_cps(src, dst, j0, j1, k, rows=slice(None)):
            return [cp(src.at[rows, j * 128:(j + 1) * 128], dst.at[j, rows], k) for j in range(j0, j1)]

        def start(cs):
            for c_ in cs:
                c_.start()

        def wait(cs):
            for c_ in cs:
                c_.wait()

        def wm_cp(p):
            return cp(wmod_hbm.at[:, pl.ds(pl.multiple_of(p * 512, 512), 512)], wm_v.at[p], 14 + p)

        def wmc_cp(c):
            col = pl.multiple_of(2 * D + c * 512, 512)
            return pltpu.make_async_copy(wmod_hbm.at[:, pl.ds(col, 512)], wmc_v.at[c], msem.at[c])

        c_cp = cp(c_hbm, c_v, 0)
        x0_cp = cp(x_hbm.at[0:TM], x_v.at[0:TM], 1)
        x1_cp = cp(x_hbm.at[TM:2 * TM], x_v.at[TM:2 * TM], 2)
        x2_cp = cp(x_hbm.at[2 * TM:3 * TM], x_v.at[2 * TM:3 * TM], 3)
        x3_cp = cp(x_hbm.at[3 * TM:S], x_v.at[3 * TM:S], 4)
        wq_cps = tile_cps(wqkv_hbm, wqkv_v, 0, 8, 5)
        wk_cps = [tile_cps(wqkv_hbm, wqkv_v, 8, 16, 6 + hh, pl.ds(hh * 512, 512)) for hh in range(2)]
        wv_cps = [tile_cps(wqkv_hbm, wqkv_v, 16, 24, 8 + hh, pl.ds(hh * 512, 512)) for hh in range(2)]
        wo_cps = tile_cps(wo_hbm, wo_v, 0, DT, 10)
        w1_cps = tile_cps(w1_hbm, w1_v, 0, F // 128, 11)
        w3_cps = tile_cps(w3_hbm, w3_v, 0, F // 128, 12)
        w2_cps = tile_cps(w2_hbm, w2_v, 0, DT, 13)

        start([c_cp, x0_cp] + wq_cps + [wm_cp(p_) for p_ in range(4)] + wk_cps[0] + wk_cps[1])

        wqkv_i, wo_i = wqkv_v.bitcast(i32), wo_v.bitcast(i32)
        w1_i, w3_i, w2_i = w1_v.bitcast(i32), w3_v.bitcast(i32), w2_v.bitcast(i32)

        halo_v[...] = jnp.zeros((16, HALO, 128), f32)
        acc_v[...] = jnp.zeros_like(acc_v)
        z_s[0] = jnp.int32(0)

        c_cp.wait()
        cf = c_v[...].astype(f32)
        sf = (cf * jax.nn.sigmoid(cf)).astype(bf16)
        sc16 = jnp.broadcast_to(sf, (16, D))
        sf = sf.astype(f32)
        for t in range(DT):
            ct_v[t * 128:(t + 1) * 128, :] = jnp.broadcast_to(sf[:, t * 128:(t + 1) * 128], (128, 128)).T

        def pinned(w, pin):
            if pin is None:
                return w
            z = jnp.full((8, 128), z_s[0], i32)
            return jnp.concatenate([w[0:8] | (pltpu.bitcast(pin, i32) & z), w[8:]], axis=0)

        def mm(lhs, wi, j, pin=None):
            return jnp.dot(lhs, pltpu.bitcast(pinned(wi[j], pin), bf16), preferred_element_type=f32)

        def mod(k):
            if k >= 2:
                return jnp.concatenate([modc_v[(k - 2) * 8 + j, 0:1, :] for j in range(DT)], axis=1)
            return jnp.concatenate([mod_v[2 * k, 0:1, :], mod_v[2 * k + 1, 0:1, :]], axis=1)

        def ln1_val(t):
            r = pl.ds(pl.multiple_of(t * TM, TM), TM)
            return _pack((_normalize(x_v[r, :].astype(f32)) * mod(1) + mod(0)).astype(bf16))

        def ln_pins(hw):
            rp = hw[0].shape[0] // 8
            return [_or_all([t[n * rp:(n + 1) * rp] for t in hw]) for n in range(8)]

        def st_tiles(dst, tiles, rows=slice(None)):
            for j, t in enumerate(tiles):
                dst[j, rows, :] = t

        def o_phase(t, pins):
            r = pl.ds(pl.multiple_of(t * TM, TM), TM)
            o = _ld(o_i)
            for n in range(DT):
                y_v[r, n * 128:(n + 1) * 128] = mm(o, wo_i, n, pins[n])

        def kv_tile(h, sec, n, pin=None):
            y = mm(h, wqkv_i, 8 * sec + n, pin)
            full = jnp.concatenate([halo_v[8 * (sec - 1) + n], y], axis=0)
            halo_v[8 * (sec - 1) + n] = y[TM - HALO:]
            return full

        def mod_chunk(c):
            w = wmc_v[c].astype(f32)
            outs = []
            for e in range(4):
                p = w[:, e * 128:(e + 1) * 128] * ct_v[...]
                acc = None
                for r in range(0, D, 8):
                    acc = p[r:r + 8] if acc is None else acc + p[r:r + 8]
                for s in (4, 2, 1):
                    acc = acc + pltpu.roll(acc, s, 0)
                outs.append(pltpu.bitcast(acc, i32))
                tau = c * 4 + e
                modc_v[tau] = acc + jnp.where(tau // 8 == 2, 1.0, 0.0)
            return outs

        with sc('prologue'):
            wait(wq_cps)
            _permute_cols(wqkv_i, 0, PG)
            x0_cp.wait()
            y_v[0:TM, :] = _normalize(x_v[0:TM, :].astype(f32))

            def mbody(t, carry):
                wm_cp(t).wait()

                @pl.when(t == 1)
                def _():
                    start([x1_cp] + wv_cps[0])
                r = jnp.dot(sc16, wm_v[t], preferred_element_type=f32)[0:8]
                mod_v[t] = r + jnp.where(t >= 2, 1.0, 0.0)
                return carry
            lax.fori_loop(0, 4, mbody, 0)

        with sc('A0'):
            _st(h_i, (y_v[0:TM, :] * mod(1) + mod(0)).astype(bf16))
            h = _ld(h_i)
            q = []
            for n in range(8):
                if n == 3:
                    wait(wk_cps[0])
                    start(wv_cps[1])
                    _permute_cols(wqkv_i, 8, PG, 0, 256)
                if n == 6:
                    wait(wk_cps[1])
                    start(wo_cps)
                    _permute_cols(wqkv_i, 8, PG, 256, 512)
                q.append(mm(h, wqkv_i, n))
            x1_cp.wait()
            hn = ln1_val(1)
            lp = ln_pins(hn)
            pins = [None, lp[0] | lp[1], lp[2] | lp[3] | lp[4], lp[5] | lp[6] | lp[7]] + [None] * 4
            kfull = []
            acc0 = [None] * W
            for n in range(8):
                if n == 4:
                    acc0 = _qk_products(q, kfull, range(0, 2), acc0)
                    wait(wv_cps[0])
                    _permute_cols(wqkv_i, 16, PG, 0, 256)
                if n == 6:
                    acc0 = _qk_products(q, kfull, range(2, 3), acc0)
                    wait(wv_cps[1])
                    start([x2_cp, wmc_cp(0), x3_cp])
                    _permute_cols(wqkv_i, 16, PG, 256, 512)
                kfull.append(kv_tile(h, 1, n, pins[n]))
            ps, inv = _softmax_weights(q, kfull, 0, acc0, range(3, DT))
            vfull = []
            for n in range(8):
                pin = None
                if n == 4:
                    wait(wo_cps)
                    rpins = _permute_rows(wo_i)
                if 1 <= n < 4:
                    pin = _or_all([inv[(n - 1) * TM // 3 // 8 * 8:n * TM // 3 // 8 * 8]])
                elif n >= 5:
                    pin = _or_all(rpins[(n - 5) * 8 // 3:(n - 4) * 8 // 3])
                vfull.append(kv_tile(h, 2, n, pin))
            of = [_pv(ps, vfull[j]) for j in range(DT)]
            _st(o_i, jnp.concatenate([o_.astype(bf16) for o_ in of], axis=1))
            st_tiles(h_i, hn)

        def a_body(i, carry):
            wmc_cp(i - 1).wait()
            for it_, waits, starts in ((1, [x2_cp], [wmc_cp(c) for c in range(1, 8)]),
                                       (2, [x3_cp], w1_cps), (4, [], w3_cps), (6, [], w2_cps)):
                @pl.when(i == it_)
                def _(waits=waits, starts=starts):
                    wait(waits)
                    start(starts)

            with sc('Ait'):
                h = _ld(h_i)
                mp = mod_chunk(i - 1)
                hn = ln1_val(jnp.minimum(i + 1, NT - 1))
                lp = ln_pins(hn)
                qp = [None] + lp[0:6] + [lp[6] | lp[7]]
                q = [mm(h, wqkv_i, n, qp[n]) for n in range(8)]
                kfull = [kv_tile(h, 1, n) for n in range(8)]
                ps, _ = _softmax_weights(q, kfull, i * TM)
                vfull = [kv_tile(h, 2, n) for n in range(8)]
                of = [_pv(ps, vfull[j]) for j in range(DT)]
                op = [_or_all([of[n]]) for n in range(DT)]
                op = [op[n] | mp[n - 2] if 2 <= n < 6 else op[n] for n in range(DT)]
                o_phase(i - 1, op)
                _st(o_i, jnp.concatenate([o_.astype(bf16) for o_ in of], axis=1))
                st_tiles(h_i, hn)
            return carry
        lax.fori_loop(1, NT, a_body, 0)

        with sc('wo7'):
            pltpu.make_async_copy(w1_v, w1_v, sems.at[11]).wait()
            pltpu.make_async_copy(w3_v, w3_v, sems.at[12]).wait()
            pltpu.make_async_copy(w2_v, w2_v, sems.at[13]).wait()
            wmc_cp(7).wait()
            x10 = x_v[0:TM, :].astype(f32) + mod(2) * y_v[0:TM, :]
            h20 = _pack((_normalize(x10) * mod(4) + mod(3)).astype(bf16))
            mp = mod_chunk(7)
            lp = ln_pins(h20)
            o_phase(NT - 1, [None, lp[0] | lp[1], lp[2] | lp[3], lp[4] | lp[5], lp[6] | lp[7],
                             mp[0] | mp[1], mp[2] | mp[3], None])
            st_tiles(h2_i.at[0], h20)

        def f_body(it, carry):
            with sc('Fit'):
                i = it // 2
                half = it % 2
                r = pl.ds(pl.multiple_of(i * TM, TM), TM)
                h2 = _ld(h2_i.at[i % 2])
                hm = TM // 2
                t = jnp.minimum(i + 1, NT - 1)
                rr = pl.ds(pl.multiple_of(t * TM + half * hm, hm), hm)
                xn = x_v[rr, :].astype(f32) + mod(2) * y_v[rr, :]
                hn = _pack((_normalize(xn) * mod(4) + mod(3)).astype(bf16))
                lp = ln_pins(hn)
                nt = FH // 128
                t0 = half * nt
                w1 = jnp.concatenate([pltpu.bitcast(pinned(w1_i[t0 + e], lp[e - 2] if 2 <= e < 10 else None), bf16)
                                      for e in range(nt)], axis=1)
                w3 = jnp.concatenate([pltpu.bitcast(w3_i[t0 + e], bf16) for e in range(nt)], axis=1)
                g = jnp.dot(h2, w1, preferred_element_type=f32)
                u = jnp.dot(h2, w3, preferred_element_type=f32)
                a = (_silu(g) * u).astype(bf16)
                kr = pl.ds(pl.multiple_of(t0 * 64, 64), FH // 2)
                w2 = jnp.concatenate([pltpu.bitcast(w2_i[j, kr, :], bf16) for j in range(DT)], axis=1)
                acc = jnp.where(half == 1, acc_v[...], 0.0) + jnp.dot(a, w2, preferred_element_type=f32)
                acc_v[...] = acc
                x1 = x_v[r, :].astype(f32) + mod(2) * y_v[r, :]
                out_v[r, :] = (x1 + mod(5) * acc).astype(out_v.dtype)
                st_tiles(h2_i.at[(i + 1) % 2], hn, rows=pl.ds(pl.multiple_of(half * (hm // 2), hm // 2), hm // 2))

                @pl.when(half == 1)
                def _():
                    pltpu.make_async_copy(out_v.at[r], out_hbm.at[r], osem.at[i]).start()
            return carry
        lax.fori_loop(0, 2 * NT, f_body, 0)

        with sc('tail'):
            for i in range(NT):
                r = pl.ds(i * TM, TM)
                pltpu.make_async_copy(out_v.at[r], out_hbm.at[r], osem.at[i]).wait()

    return kernel


def build(debug=False, scopes=False):
    odt = f32 if debug else bf16

    def f(A_x, A_wqkv, A_wo, B_w1, B_w3, B_w2, c, w_mod):
        x = A_x.reshape(S, D)
        anyspec = pl.BlockSpec(memory_space=pl.ANY)
        out = pl.pallas_call(
            make_kernel(scopes),
            in_specs=[anyspec] * 8,
            out_specs=anyspec,
            out_shape=jax.ShapeDtypeStruct((S, D), odt),
            scratch_shapes=[
                pltpu.VMEM((S, D), bf16),
                pltpu.VMEM((3 * DT, D, 128), bf16),
                pltpu.VMEM((DT, D, 128), bf16),
                pltpu.VMEM((F // 128, D, 128), bf16),
                pltpu.VMEM((F // 128, D, 128), bf16),
                pltpu.VMEM((DT, F, 128), bf16),
                pltpu.VMEM((1, D), bf16),
                pltpu.VMEM((4, D, 512), bf16),
                pltpu.VMEM((8, D, 512), bf16),
                pltpu.VMEM((4, 8, 512), f32),
                pltpu.VMEM((32, 8, 128), f32),
                pltpu.VMEM((D, 128), f32),
                pltpu.VMEM((DT, TM // 2, 128), i32),
                pltpu.VMEM((DT, TM // 2, 128), i32),
                pltpu.VMEM((16, HALO, 128), f32),
                pltpu.VMEM((S, D), f32),
                pltpu.VMEM((2, DT, TM // 2, 128), i32),
                pltpu.VMEM((TM, D), f32),
                pltpu.VMEM((S, D), odt),
                pltpu.SemaphoreType.DMA((18,)),
                pltpu.SemaphoreType.DMA((NT,)),
                pltpu.SemaphoreType.DMA((8,)),
                pltpu.SMEM((1,), i32),
            ],
            compiler_params=pltpu.CompilerParams(vmem_limit_bytes=100 * 2**20),
        )(x, A_wqkv, A_wo, B_w1, B_w3, B_w2, c, w_mod)
        return out.reshape(1, S, D)
    return f


@jax.jit
def pallas_adaLN_cond__sliding_local_dilated__glu_gated_swiglu__prompt_kernel(
    A_x: jax.Array,
    A_wqkv: jax.Array,
    A_wo: jax.Array,
    B_x: jax.Array,
    B_w1: jax.Array,
    B_w3: jax.Array,
    B_w2: jax.Array,
    c: jax.Array,
    w_mod: jax.Array,
):
    del B_x
    return build()(A_x, A_wqkv, A_wo, B_w1, B_w3, B_w2, c, w_mod)
```
